```python
import os as _os
_os.environ.setdefault("JAX_PLATFORMS", "cpu")
import jax
import jax.numpy as jnp

def _softmax(x, axis=-1):
    return jax.nn.softmax(x, axis=axis)
def _gelu(x):
    return jax.nn.gelu(x, approximate=True)
def _silu(x):
    return jax.nn.silu(x)
def _sigmoid(x):
    return jax.nn.sigmoid(x)
def _layernorm(x, axis=-1, eps=1e-5):
    m = jnp.mean(x, axis=axis, keepdims=True)
    v = jnp.var(x, axis=axis, keepdims=True)
    return (x - m) / jnp.sqrt(v + eps)
def _scatter_add(tgt, idx, src, axis=0):
    return tgt.at[idx].add(src)
def _segment_sum(src, seg, n):
    return jax.ops.segment_sum(src, seg, n)
class _Rng:
    def __init__(self, key):
        self._k = key
    def _next(self):
        self._k, sub = jax.random.split(self._k)
        return sub
    def normal(self, shape):
        return jax.random.normal(self._next(), shape, dtype=jnp.bfloat16)
    def randint(self, lo, hi, shape):
        return jax.random.randint(self._next(), shape, lo, hi, dtype=jnp.int32)
    def uniform(self, shape, lo=0.0, hi=1.0):
        return jax.random.uniform(self._next(), shape, jnp.bfloat16, lo, hi)
    def permutation(self, n):
        return jax.random.permutation(self._next(), n)


kernel_name = 'gated_mix__linear_kernel_hedgehog__mixer_s_mlp__prompt'

def setup_inputs():
    _rng = _Rng(jax.random.key(int.from_bytes(__import__("os").urandom(4), "little")))
    _w = (lambda a: (lambda t: t.astype(jnp.bfloat16) if jnp.issubdtype(t.dtype, jnp.floating) else t)(jnp.asarray(a)))
    def _A_setup():
        B, S, D, H = 1, 2048, 512, 32
        Dh = D // H
        return {
            "x": _w((lambda *s: _rng.normal(s) * 0.05)(B, S, D)),
            "wqkv": _w((lambda *s: _rng.normal(s) * 1.6)(D, 3 * D)),
            "w_phi": _w((lambda *s: _rng.normal(s) * 1.6)(H, Dh, Dh) * (Dh ** -0.5)),
            "wo": _w((lambda *s: _rng.normal(s) * 0.05)(D, D)),
        }
    _A_in = _A_setup()

    def _B_setup():
        B, S, D, F = 1, 2048, 512, 1376
        return {
            "x":  _w((lambda *s: _rng.normal(s) * 0.05)(B, S, D)),
            "w1": _w((lambda *s: _rng.normal(s) * 0.4)(D, D) * (D ** -0.5)),
            "w2": _w((lambda *s: _rng.normal(s) * 0.4)(D, D) * (D ** -0.5)),
            "w3": _w((lambda *s: _rng.normal(s) * 0.4)(D, F) * (D ** -0.5)),
            "w4": _w((lambda *s: _rng.normal(s) * 0.4)(F, D) * (F ** -0.5)),
        }
    _B_in = _B_setup()

    return {
        "A_x": _A_in["x"],
        "A_wqkv": _A_in["wqkv"],
        "A_w_phi": _A_in["w_phi"],
        "A_wo": _A_in["wo"],
        "B_x": _B_in["x"],
        "B_w1": _B_in["w1"],
        "B_w2": _B_in["w2"],
        "B_w3": _B_in["w3"],
        "B_w4": _B_in["w4"],
        "gate_w": _w((lambda *s: _rng.normal(s) * 0.05)(512) * 16.0),
    }

def reference(A_x, A_wqkv, A_w_phi, A_wo, B_x, B_w1, B_w2, B_w3, B_w4, gate_w):
    def _A_ref(x, wqkv, w_phi, wo):
        B, S, D = x.shape
        H = 32; Dh = D // H
        qkv = (lambda x, *d: x.transpose(*d))((x @ wqkv).reshape(B, S, 3, H, Dh), 2, 0, 3, 1, 4)
        q, k, v = qkv[0], qkv[1], qkv[2]
        pq = jnp.einsum("bhsd,hdf->bhsf", q, w_phi)
        pk = jnp.einsum("bhsd,hdf->bhsf", k, w_phi)
        phi_q = jnp.concatenate([_softmax(pq, axis=-1), _softmax(-pq, axis=-1)], axis=-1)
        phi_k = jnp.concatenate([_softmax(pk, axis=-1), _softmax(-pk, axis=-1)], axis=-1)
        kv = jnp.einsum("bhsf,bhsd->bhfd", phi_k, v)
        z  = jnp.einsum("bhsf->bhf", phi_k)
        num = jnp.einsum("bhqf,bhfd->bhqd", phi_q, kv)
        den = jnp.einsum("bhqf,bhf->bhq", phi_q, z)[..., None] + 1e-6
        o = num / den
        return (lambda x, *d: x.transpose(*d))(o, 0, 2, 1, 3).reshape(B, S, D) @ wo

    def _B_ref(x, w1, w2, w3, w4):
        B, S, D = x.shape
        h = _gelu(_layernorm(x, axis=-1) @ w1)
        c = D // 4
        g0 = jnp.pad(h[:, :, 0*c:1*c], ((0, 0), (1, 0), (0, 0)))[:, :S, :]
        g1 = jnp.pad(h[:, :, 1*c:2*c], ((0, 0), (0, 1), (0, 0)))[:, 1:, :]
        g2 = jnp.pad(h[:, :, 2*c:3*c], ((0, 0), (2, 0), (0, 0)))[:, :S, :]
        g3 = jnp.pad(h[:, :, 3*c:   ], ((0, 0), (0, 2), (0, 0)))[:, 2:, :]
        hs = jnp.concatenate([g0, g1, g2, g3], axis=-1) @ w2
        x1 = x + hs
        h2 = _gelu(_layernorm(x1, axis=-1) @ w3) @ w4
        return x1 + h2

    x = A_x
    g = _sigmoid((x * gate_w).sum(-1, keepdims=True))
    a = _A_ref(x, A_wqkv, A_w_phi, A_wo)
    b = _B_ref(x, B_w1, B_w2, B_w3, B_w4)
    return g * a + (1 - g) * b
```

```python
import functools
import jax
import jax.numpy as jnp
from jax import lax
import jax.experimental.pallas as pl
import jax.experimental.pallas.tpu as pltpu

S, D, H, DH, F = 2048, 512, 32, 16, 1376
TS = 256
NT = S // TS
G = 8
PAD = 8
LOG2E = 1.4426950408889634
NTD = (((1,), (1,)), ((), ()))
TND = (((0,), (0,)), ((), ()))
f32 = jnp.float32
bf16 = jnp.bfloat16


def _gelu(x):
    c = 0.7978845608028654
    inner = x * (c + (c * 0.044715) * (x * x))
    hx = 0.5 * x
    return hx + hx * jnp.tanh(inner)


def _ln(x):
    m = jnp.mean(x, axis=-1, keepdims=True)
    xc = x - m
    v = jnp.mean(xc * xc, axis=-1, keepdims=True)
    return xc * lax.rsqrt(v + 1e-5)


def _phi_t(p):
    T = p.shape[-1]
    p3 = p.reshape(8, 8, T)
    mx = jnp.max(p3, axis=0)
    mn = jnp.min(p3, axis=0)
    mx = jnp.maximum(mx, pltpu.roll(mx, 4, 0))
    mn = jnp.minimum(mn, pltpu.roll(mn, 4, 0))
    ep = jnp.exp2(p3 - mx[None])
    en = jnp.exp2(mn[None] - p3)
    sp = jnp.sum(ep, axis=0)
    sn = jnp.sum(en, axis=0)
    rp = 1.0 / (sp + pltpu.roll(sp, 4, 0))
    rn = 1.0 / (sn + pltpu.roll(sn, 4, 0))
    return jnp.concatenate([(ep * rp[None]).reshape(64, T).astype(bf16),
                            (en * rn[None]).reshape(64, T).astype(bf16)], axis=0)


def _iota(shape, dim):
    return lax.broadcasted_iota(jnp.int32, shape, dim)


def _kernel(x_hbm, wqkv_hbm, wphi_ref, wo_hbm, w1_hbm, w2_hbm, w3t_hbm, w4_hbm, gw_ref, o_hbm,
            x_ref, wqkv_ref, wo_ref, w1_ref, w2_ref, w3t_ref, w4_ref, o_ref,
            wt_ref, wop_ref, kv_ref, kvb_ref, h_ref, xsem, wsem, osem):
    def x_copy(t):
        return pltpu.make_async_copy(x_hbm.at[pl.ds(t * TS, TS), :], x_ref.at[pl.ds(t * TS, TS), :], xsem.at[t])

    def o_copy(t):
        return pltpu.make_async_copy(o_ref.at[pl.ds(t * TS, TS), :], o_hbm.at[pl.ds(t * TS, TS), :], osem.at[t])

    c_k = pltpu.make_async_copy(wqkv_hbm.at[:, 512:1024], wqkv_ref.at[:, 512:1024], wsem.at[0])
    c_v = pltpu.make_async_copy(wqkv_hbm.at[:, 1024:1536], wqkv_ref.at[:, 1024:1536], wsem.at[1])
    c_q = pltpu.make_async_copy(wqkv_hbm.at[:, 0:512], wqkv_ref.at[:, 0:512], wsem.at[2])
    c_w1 = pltpu.make_async_copy(w1_hbm, w1_ref, wsem.at[3])
    c_wo = pltpu.make_async_copy(wo_hbm, wo_ref, wsem.at[4])
    c_w2 = pltpu.make_async_copy(w2_hbm, w2_ref, wsem.at[5])
    c_w3 = pltpu.make_async_copy(w3t_hbm, w3t_ref, wsem.at[6])
    c_w4 = pltpu.make_async_copy(w4_hbm, w4_ref, wsem.at[7])

    c_k.start()
    c_v.start()
    x_copy(0).start()
    c_w1.start()
    for t in range(1, NT):
        x_copy(t).start()
    c_q.start()
    c_wo.start()
    c_w2.start()
    c_w3.start()
    c_w4.start()

    w2d = wphi_ref[...].reshape(256, 32)
    rep = jnp.where(_iota((32, 512), 0) == _iota((32, 512), 1) // 16, 1.0, 0.0).astype(bf16)
    cc = jnp.dot(w2d, rep, preferred_element_type=f32)
    cc = jnp.where(_iota((256, 512), 0) // 16 == _iota((256, 512), 1) % 16, cc, 0.0).astype(bf16)
    sel = jnp.where((_iota((128, 256), 0) % 64) // 4 == _iota((128, 256), 1) % 16, 1.0, 0.0).astype(bf16)
    et = jnp.dot(sel, cc, preferred_element_type=f32)
    r = _iota((128, 512), 0)
    hh8 = (r // 64) * 4 + r % 4
    bdt = jnp.where(hh8 == (_iota((128, 512), 1) // 16) % 8, et, 0.0).astype(bf16)
    r = _iota((128, 128), 0)
    perm = jnp.where(((r // 64) * 4 + r % 4) * 16 + (r % 64) // 4 == _iota((128, 128), 1), 1.0, 0.0).astype(bf16)

    kv_ref[...] = jnp.zeros_like(kv_ref)
    h_ref[:, 0:PAD, :] = jnp.zeros((4, PAD, 128), f32)
    h_ref[:, PAD + S:PAD + S + PAD, :] = jnp.zeros((4, PAD, 128), f32)

    def fold(j):
        for g in range(4):
            lo = j * 512 + g * 128
            wt_ref[lo:lo + 128, :] = (lax.dot_general(
                bdt[:, g * 128:(g + 1) * 128], wqkv_ref[:, lo:lo + 128], NTD,
                preferred_element_type=f32) * LOG2E).astype(bf16)

    c_k.wait()
    fold(1)
    c_v.wait()
    for g in range(4):
        lo = 1024 + g * 128
        wt_ref[lo:lo + 128, :] = lax.dot_general(
            perm, wqkv_ref[:, lo:lo + 128], NTD, preferred_element_type=f32).astype(bf16)
    c_w1.wait()

    def p1(t, carry):
        x_copy(t).wait()
        r0 = pl.multiple_of(t * TS, TS)
        x = x_ref[pl.ds(r0, TS), :]
        kvt = lax.dot_general(wt_ref[512:1536, :], x, NTD, preferred_element_type=f32)
        ones = jnp.ones((16, TS), bf16)
        for g in range(G):
            phi = _phi_t(kvt[g * 64:(g + 1) * 64, :])
            vt = jnp.concatenate([kvt[512 + g * 64: 512 + (g + 1) * 64, :].astype(bf16), ones], axis=0)
            kv_ref[g] += lax.dot_general(vt, phi, NTD, preferred_element_type=f32)
        y = _ln(x.astype(f32)).astype(bf16)
        h = _gelu(jnp.dot(y, w1_ref[...], preferred_element_type=f32))
        h0 = pl.multiple_of(PAD + t * TS, 8)
        for j in range(4):
            h_ref[j, pl.ds(h0, TS), :] = h[:, j * 128:(j + 1) * 128]
        return carry

    lax.fori_loop(0, NT, p1, 0)

    c_q.wait()
    c_wo.wait()
    c_w2.wait()
    c_w3.wait()
    c_w4.wait()
    fold(0)
    for g in range(4):
        sl = slice(g * 128, (g + 1) * 128)
        wop_ref[sl, :] = jnp.dot(perm, wo_ref[sl, :], preferred_element_type=f32).astype(bf16)
    mask = (_iota((80, 128), 0) % 4) == (_iota((80, 128), 1) % 4)
    for g in range(G):
        kvb_ref[g] = jnp.where(mask, kv_ref[g], 0.0).astype(bf16)
    gw = gw_ref[...].astype(f32).reshape(1, D)

    def p2(t, carry):
        r0 = pl.multiple_of(t * TS, TS)
        x = x_ref[pl.ds(r0, TS), :]
        qt = lax.dot_general(wt_ref[0:512, :], x, NTD, preferred_element_type=f32)
        ots = []
        for g in range(G):
            phi = _phi_t(qt[g * 64:(g + 1) * 64, :])
            nt = jnp.dot(kvb_ref[g], phi, preferred_element_type=f32)
            rden = 1.0 / (nt[64:72, :] + 1e-6)
            ots.append((nt[0:64, :].reshape(8, 8, TS) * rden[None]).reshape(64, TS).astype(bf16))
        ot = jnp.concatenate(ots, axis=0)
        a = lax.dot_general(ot, wop_ref[...], TND, preferred_element_type=f32)
        xf = x.astype(f32)
        base = PAD + t * TS
        hs = jnp.concatenate([h_ref[j, pl.ds(base + off, TS), :].astype(bf16)
                              for j, off in enumerate((-1, 1, -2, 2))], axis=1)
        x1 = xf + jnp.dot(hs, w2_ref[...], preferred_element_type=f32)
        y = _ln(x1).astype(bf16)
        u = _gelu(lax.dot_general(y, w3t_ref[...], NTD, preferred_element_type=f32)).astype(bf16)
        b = x1 + jnp.dot(u, w4_ref[...], preferred_element_type=f32)
        gate = jax.nn.sigmoid(jnp.sum(xf * gw, axis=-1, keepdims=True))
        o_ref[pl.ds(r0, TS), :] = (b + gate * (a - b)).astype(bf16)
        o_copy(t).start()
        return carry

    lax.fori_loop(0, NT, p2, 0)
    for t in range(NT):
        o_copy(t).wait()


@jax.jit
def pallas_gated_mix__linear_kernel_hedgehog__mixer_s_mlp__prompt_kernel(
    A_x, A_wqkv, A_w_phi, A_wo, B_x, B_w1, B_w2, B_w3, B_w4, gate_w):
    x = A_x.reshape(S, D)
    wphi = jnp.transpose(A_w_phi, (1, 2, 0))
    w3t = B_w3.T
    hbm = pl.BlockSpec(memory_space=pl.ANY)
    vmem = pl.BlockSpec(memory_space=pltpu.VMEM)
    out = pl.pallas_call(
        _kernel,
        in_specs=[hbm, hbm, vmem, hbm, hbm, hbm, hbm, hbm, vmem],
        out_specs=hbm,
        out_shape=jax.ShapeDtypeStruct((S, D), bf16),
        scratch_shapes=[
            pltpu.VMEM((S, D), bf16),
            pltpu.VMEM((D, 3 * D), bf16),
            pltpu.VMEM((D, D), bf16),
            pltpu.VMEM((D, D), bf16),
            pltpu.VMEM((D, D), bf16),
            pltpu.VMEM((F, D), bf16),
            pltpu.VMEM((F, D), bf16),
            pltpu.VMEM((S, D), bf16),
            pltpu.VMEM((1536, 512), bf16),
            pltpu.VMEM((512, 512), bf16),
            pltpu.VMEM((G, 80, 128), f32),
            pltpu.VMEM((G, 80, 128), bf16),
            pltpu.VMEM((4, S + 2 * PAD, 128), f32),
            pltpu.SemaphoreType.DMA((NT,)),
            pltpu.SemaphoreType.DMA((8,)),
            pltpu.SemaphoreType.DMA((NT,)),
        ],
        compiler_params=pltpu.CompilerParams(vmem_limit_bytes=100 * 1024 * 1024),
    )(x, A_wqkv, wphi, A_wo, B_w1, B_w2, w3t, B_w4, gate_w)
    return out.reshape(1, S, D)
```

```python
import functools

import jax
import jax.numpy as jnp
from jax import lax
import jax.experimental.pallas as pl
import jax.experimental.pallas.tpu as pltpu

S, D, H, DH, F = 2048, 512, 32, 16, 1376
G = 8
FM = 1280
PAD = 8
T2 = 1024
TP = 256
KA = 3
XA, XB, XC = 256, 512, 768
LOG2E = 1.4426950408889634

f32 = jnp.float32
bf16 = jnp.bfloat16
u32 = jnp.uint32

_nn = functools.partial(jnp.dot, preferred_element_type=f32)
_nt = functools.partial(lax.dot_general, dimension_numbers=(((1,), (1,)), ((), ())),
                        preferred_element_type=f32)
_tn = functools.partial(lax.dot_general, dimension_numbers=(((0,), (0,)), ((), ())),
                        preferred_element_type=f32)


def _gelu(x):
    c = 0.7978845608028654
    inner = x * (c + (c * 0.044715) * (x * x))
    hx = 0.5 * x
    return hx + hx * jnp.tanh(inner)


def _ln_stats(x):
    m = jnp.mean(x, axis=-1, keepdims=True)
    xc = x - m
    v = jnp.mean(xc * xc, axis=-1, keepdims=True)
    return m, xc, lax.rsqrt(v + 1e-5)


def _fold4(v, op):
    return op(v, pltpu.roll(v, 4, 0))


def _exps(p):
    p3 = p.reshape(8, 8, p.shape[-1])
    mx = _fold4(jnp.max(p3, axis=0), jnp.maximum)
    mn = _fold4(jnp.min(p3, axis=0), jnp.minimum)
    ep = jnp.exp2(p3 - mx[None])
    en = jnp.exp2(mn[None] - p3)
    sp = _fold4(jnp.sum(ep, axis=0), jnp.add)
    sn = _fold4(jnp.sum(en, axis=0), jnp.add)
    return ep, en, sp, sn


def _iota(shape, dim):
    return lax.broadcasted_iota(jnp.int32, shape, dim)


def _kernel(x_hbm, wqkv_hbm, wphi_hbm, wo_hbm, w1_hbm, w2_hbm, w3t_hbm, w4_hbm, gw_hbm, o_hbm,
            x_ref, wqkv_ref, wphi_ref, wo_ref, w1_ref, w2_ref, w3t_ref, w4_ref, gw_ref, o_ref,
            wt_ref, kv_ref, kvb_ref, z_ref, h_ref, sem):
    cp = pltpu.make_async_copy

    def w_cols(a, b, s):
        return cp(wqkv_hbm.at[:, a:b], wqkv_ref.at[:, a:b], sem.at[s])

    def x_rows(a, b, s):
        return cp(x_hbm.at[a:b, :], x_ref.at[a:b, :], sem.at[s])

    def start(cs):
        for c in cs:
            c.start()

    def wait(cs):
        for c in cs:
            c.wait()

    ka_end = D + 128 * KA
    g0 = [cp(wphi_hbm, wphi_ref, sem.at[0])]
    g1 = [w_cols(D, ka_end, 1)]
    g2 = [x_rows(0, XA, 2)]
    g3 = [w_cols(ka_end, 2 * D, 3), x_rows(XA, XB, 3)]
    g4 = [w_cols(2 * D, 3 * D, 4), x_rows(XB, XC, 4)]
    g5 = [cp(w1_hbm, w1_ref, sem.at[0]), x_rows(XC, S, 0), w_cols(0, D, 0)]
    g6 = [cp(gw_hbm, gw_ref, sem.at[1]), cp(w2_hbm, w2_ref, sem.at[1]), cp(wo_hbm, wo_ref, sem.at[1]),
          cp(w3t_hbm, w3t_ref, sem.at[1]), cp(w4_hbm, w4_ref, sem.at[1])]
    start(g0 + g1 + g2 + g3 + g4)

    h_ref[:, 0:PAD, :] = jnp.zeros((4, PAD, 128), f32)
    h_ref[:, PAD + S:PAD + S + PAD, :] = jnp.zeros((4, PAD, 128), f32)

    rep = jnp.where(_iota((32, 512), 0) == _iota((32, 512), 1) // 16, 1.0, 0.0).astype(bf16)
    m1 = _iota((256, 128), 0) // 16 == _iota((256, 128), 1) % 16
    sel = jnp.where((_iota((128, 256), 0) % 64) // 4 == _iota((128, 256), 1) % 16, 1.0, 0.0).astype(bf16)
    r = _iota((128, 128), 0)
    m2 = (r // 64) * 4 + r % 4 == _iota((128, 128), 1) // 16
    wait(g0)
    start(g5)
    w2d = wphi_ref[...].reshape(256, 32)
    cc = _nn(w2d, rep)
    cc = jnp.where(jnp.concatenate([m1] * 4, axis=1), cc, 0.0).astype(bf16)
    et = _nn(sel, cc)
    bdt = jnp.where(jnp.concatenate([m2] * 4, axis=1), et, 0.0).astype(bf16)

    def fold(j, blocks):
        for b in blocks:
            lo = j * D + b * 128
            wt_ref[lo // 2:lo // 2 + 64, :] = pltpu.bitcast(
                (_nt(bdt[:, b * 128:(b + 1) * 128], wqkv_ref[:, lo:lo + 128]) * LOG2E).astype(bf16), u32)

    def wt(a, b):
        return pltpu.bitcast(wt_ref[a // 2:b // 2, :], bf16)

    def k_phi(kt):
        t = kt.shape[-1]
        ep, en, sp, sn = _exps(kt)
        phi = jnp.concatenate([(ep * (1.0 / sp)[None]).reshape(64, t),
                               (en * (1.0 / sn)[None]).reshape(64, t)], axis=0)
        z = phi[:, 0:128]
        for c in range(1, t // 128):
            z = z + phi[:, c * 128:(c + 1) * 128]
        return phi.astype(bf16), z

    def ln1(r0, n):
        _, xc, rs = _ln_stats(x_ref[r0:r0 + n, :].astype(f32))
        return (xc * rs).astype(bf16)

    def h_rows(y, r0):
        h = _gelu(_nn(y, w1_ref[...]))
        for j in range(4):
            h_ref[j, PAD + r0:PAD + r0 + y.shape[0], :] = h[:, j * 128:(j + 1) * 128]

    phis = {}
    z_set = set()
    pending = []

    def feat(g, c, kt):
        phi, z = k_phi(kt)
        if g in z_set:
            z_ref[g] += z
        else:
            z_ref[g] = z
            z_set.add(g)
        for j in range(kt.shape[1] // 128):
            phis[(g, c + j * 128)] = phi[:, j * 128:(j + 1) * 128]

    def kproj(gs, c0, c1, defer=0):
        kt = _nt(wt(D + 64 * gs[0], D + 64 * (gs[-1] + 1)), x_ref[c0:c1, :])
        n = c1 - c0
        for i, g in enumerate(gs):
            kg = kt[i * 64:(i + 1) * 64, :]
            if i >= len(gs) - defer:
                feat(g, c0, kg[:, 0:n - 128])
                pending.append((g, c1 - 128, kg[:, n - 128:n]))
            else:
                feat(g, c0, kg)

    ga, gb = list(range(2 * KA)), list(range(2 * KA, G))
    wait(g1)
    fold(1, range(KA))
    wait(g2)
    kproj(ga, 0, XA, defer=2)
    wait(g3)
    fold(1, range(KA, 4))
    kproj(ga, XA, XB)
    kproj(gb, 0, XA)
    kproj(gb, XA, XB, defer=2)
    wait(g4)
    for p in pending:
        feat(*p)
    start(g6)
    wvt = wqkv_ref[:, 2 * D:3 * D].T
    wt_ref[D:3 * D // 2, :] = pltpu.bitcast(wvt, u32)
    kproj(ga + gb, XB, XC)
    vc = XC // 2
    for c0 in range(0, XC, vc):
        vt = _nt(wvt, x_ref[c0:c0 + vc, :]).astype(bf16)
        for g in range(G):
            ph = jnp.concatenate([phis[(g, c)] for c in range(c0, c0 + vc, 128)], axis=1)
            upd = _nt(vt[g * 64:(g + 1) * 64, :], ph)
            if c0 == 0:
                kv_ref[g] = upd
            else:
                kv_ref[g] += upd
    y0 = ln1(0, 128)
    wait(g5)

    h_rows(y0, 0)
    backlog = list(range(128, XC, 128))
    for i, r0 in enumerate(range(XC, S, TP)):
        if i == 1:
            fold(0, range(4))
        kvt = _nt(wt(D, 3 * D), x_ref[r0:r0 + TP, :])
        phs = []
        for g in range(G):
            phi, z = k_phi(kvt[g * 64:(g + 1) * 64, :])
            z_ref[g] += z
            phs.append(phi)
        vt = kvt[D:2 * D, :].astype(bf16)
        for g in range(G):
            kv_ref[g] += _nt(vt[g * 64:(g + 1) * 64, :], phs[g])
        h_rows(ln1(r0, TP), r0)
        h_rows(ln1(backlog[i], 128), backlog[i])
    head_match = (_iota((64, 128), 0) // 16) == (_iota((64, 128), 1) % 4)
    for g in range(G):
        kvb_ref[g] = pltpu.bitcast(jnp.where(head_match, kv_ref[g], 0.0).astype(bf16), u32)
    wait(g6)

    def p2(t, carry):
        r0 = pl.multiple_of(t * T2, T2)
        x = x_ref[pl.ds(r0, T2), :]
        xf = x.astype(f32)
        gw = gw_ref[...].astype(f32).reshape(1, D)
        gate = 0.5 + 0.5 * jnp.tanh(0.5 * jnp.sum(xf * gw, axis=-1, keepdims=True))

        def mix(lo, n):
            base = PAD + t * T2 + lo
            hs = jnp.concatenate([h_ref[j, pl.ds(base + off, n), :]
                                  for j, off in enumerate((-1, 1, -2, 2))], axis=1).astype(bf16)
            return xf[lo:lo + n, :] + _nn(hs, w2_ref[...])

        x1a = mix(0, T2 // 2)
        qt = _nt(wt(0, D), x)
        ots = []
        for g in range(G):
            ep, en, sp, sn = _exps(qt[g * 64:(g + 1) * 64, :])
            zb = jnp.broadcast_to(jnp.sum(z_ref[g], axis=-1, keepdims=True), (128, 128))
            z = jnp.concatenate([zb] * (T2 // 128), axis=1).reshape(16, 8, T2)
            dp = jnp.sum(ep * z[0:8], axis=0)
            dn = jnp.sum(en * z[8:16], axis=0)
            rr = 1.0 / (_fold4(dp * sn + dn * sp, jnp.add) + 1e-6 * (sp * sn))
            phi = jnp.concatenate([(ep * (sn * rr)[None]).reshape(64, T2),
                                   (en * (sp * rr)[None]).reshape(64, T2)], axis=0).astype(bf16)
            ots.append(_nn(pltpu.bitcast(kvb_ref[g], bf16), phi))
        ot = jnp.concatenate(ots, axis=0).astype(bf16)
        x1 = jnp.concatenate([x1a, mix(T2 // 2, T2 // 2)], axis=0)
        a = _tn(ot, wo_ref[...])
        m, _, rs = _ln_stats(x1)
        y = (x1 * rs - m * rs).astype(bf16)
        u = _gelu(_nt(y, w3t_ref[0:FM, :])).astype(bf16)
        ut = _gelu(_nt(w3t_ref[FM:F, :], y)).astype(bf16)
        u = jnp.concatenate([u, ut.T], axis=1)
        c = x1 + gate * (a - x1)
        og = 1.0 - gate
        for j in range(4):
            sl = slice(j * 128, (j + 1) * 128)
            ra = 0
            for rn in ([T2] if j < 3 else [512, 256, 128, 128]):
                h2 = _nn(u[ra:ra + rn, :], w4_ref[:, sl])
                rows = pl.ds(pl.multiple_of(r0 + ra, 128), rn)
                o_ref[rows, sl] = (c[ra:ra + rn, sl] + og[ra:ra + rn] * h2).astype(bf16)
                cp(o_ref.at[rows, sl], o_hbm.at[rows, sl], sem.at[2]).start()
                ra += rn
        return carry

    lax.fori_loop(0, S // T2, p2, 0)
    cp(o_ref, o_hbm, sem.at[2]).wait()


@jax.jit
def pallas_gated_mix__linear_kernel_hedgehog__mixer_s_mlp__prompt_kernel(
    A_x: jax.Array,
    A_wqkv: jax.Array,
    A_w_phi: jax.Array,
    A_wo: jax.Array,
    B_x: jax.Array,
    B_w1: jax.Array,
    B_w2: jax.Array,
    B_w3: jax.Array,
    B_w4: jax.Array,
    gate_w: jax.Array,
):
    del B_x
    x = A_x.reshape(S, D)
    wphi = jnp.transpose(A_w_phi, (1, 2, 0))
    w3t = B_w3.T
    hbm = pl.BlockSpec(memory_space=pl.ANY)
    out = pl.pallas_call(
        _kernel,
        in_specs=[hbm] * 9,
        out_specs=hbm,
        out_shape=jax.ShapeDtypeStruct((S, D), bf16),
        scratch_shapes=[
            pltpu.VMEM((S, D), bf16),
            pltpu.VMEM((D, 3 * D), bf16),
            pltpu.VMEM((DH, DH, H), bf16),
            pltpu.VMEM((D, D), bf16),
            pltpu.VMEM((D, D), bf16),
            pltpu.VMEM((D, D), bf16),
            pltpu.VMEM((F, D), bf16),
            pltpu.VMEM((F, D), bf16),
            pltpu.VMEM((D,), bf16),
            pltpu.VMEM((S, D), bf16),
            pltpu.VMEM((3 * D // 2, D), u32),
            pltpu.VMEM((G, 64, 128), f32),
            pltpu.VMEM((G, 32, 128), u32),
            pltpu.VMEM((G, 128, 128), f32),
            pltpu.VMEM((4, S + 2 * PAD, 128), f32),
            pltpu.SemaphoreType.DMA((5,)),
        ],
        compiler_params=pltpu.CompilerParams(
            vmem_limit_bytes=100 * 1024 * 1024,
            disable_bounds_checks=True,
            disable_semaphore_checks=True,
        ),
    )(x, A_wqkv, wphi, A_wo, B_w1, B_w2, w3t, B_w4, gate_w)
    return out.reshape(1, S, D)
```

```python
import functools

import jax
import jax.numpy as jnp
from jax import lax
import jax.experimental.pallas as pl
import jax.experimental.pallas.tpu as pltpu

S, D, H, DH, F = 2048, 512, 32, 16, 1376
G = 8
FM = 1280
PAD = 8
T2 = 1024
TP = 256
XC = 768
LOG2E = 1.4426950408889634

f32 = jnp.float32
bf16 = jnp.bfloat16
u32 = jnp.uint32

_nn = functools.partial(jnp.dot, preferred_element_type=f32)
_nt = functools.partial(lax.dot_general, dimension_numbers=(((1,), (1,)), ((), ())),
                        preferred_element_type=f32)
_tn = functools.partial(lax.dot_general, dimension_numbers=(((0,), (0,)), ((), ())),
                        preferred_element_type=f32)


def _gelu(x):
    c = 0.7978845608028654
    inner = x * (c + (c * 0.044715) * (x * x))
    hx = 0.5 * x
    return hx + hx * jnp.tanh(inner)


def _ln_stats(x):
    m = jnp.mean(x, axis=-1, keepdims=True)
    xc = x - m
    v = jnp.mean(xc * xc, axis=-1, keepdims=True)
    return m, xc, lax.rsqrt(v + 1e-5)


def _fold4(v, op):
    return op(v, pltpu.roll(v, 4, 0))


def _exps(p):
    p3 = p.reshape(8, 8, p.shape[-1])
    mx = _fold4(jnp.max(p3, axis=0), jnp.maximum)
    mn = _fold4(jnp.min(p3, axis=0), jnp.minimum)
    ep = jnp.exp2(p3 - mx[None])
    en = jnp.exp2(mn[None] - p3)
    sp = _fold4(jnp.sum(ep, axis=0), jnp.add)
    sn = _fold4(jnp.sum(en, axis=0), jnp.add)
    return ep, en, sp, sn


def _iota(shape, dim):
    return lax.broadcasted_iota(jnp.int32, shape, dim)


def _kernel(x_hbm, wqkv_hbm, wphi_hbm, wo_hbm, w1_hbm, w2_hbm, w3t_hbm, w4_hbm, gw_hbm, o_hbm,
            x_ref, wqkv_ref, wphi_ref, wo_ref, w1_ref, w2_ref, w3t_ref, w4_ref, gw_ref, o_ref,
            wt_ref, kv_ref, kvb_ref, z_ref, h_ref, sem):
    cp = pltpu.make_async_copy

    def w_cols(a, b, s):
        return cp(wqkv_hbm.at[:, a:b], wqkv_ref.at[:, a:b], sem.at[s])

    def x_rows(a, b, s):
        return cp(x_hbm.at[a:b, :], x_ref.at[a:b, :], sem.at[s])

    def start(cs):
        for c in cs:
            c.start()

    def wait(cs):
        for c in cs:
            c.wait()

    g0 = [cp(wphi_hbm, wphi_ref, sem.at[0])]
    g1 = [w_cols(D, D + 256, 1)]
    g2 = [x_rows(0, 128, 2)]
    g3 = [w_cols(D + 256, D + 384, 3), x_rows(128, 256, 3)]
    g4 = [w_cols(D + 384, 2 * D, 4), x_rows(256, 512, 4)]
    g5 = [w_cols(2 * D, 3 * D, 5), x_rows(512, XC, 5)]
    g6 = [cp(w1_hbm, w1_ref, sem.at[0]), x_rows(XC, S, 0), w_cols(0, D, 0)]
    g7 = [cp(gw_hbm, gw_ref, sem.at[1]), cp(w2_hbm, w2_ref, sem.at[1]), cp(wo_hbm, wo_ref, sem.at[1]),
          cp(w3t_hbm, w3t_ref, sem.at[1]), cp(w4_hbm, w4_ref, sem.at[1])]
    start(g0 + g1 + g2 + g3 + g4 + g5)

    def wt(a, b):
        return pltpu.bitcast(wt_ref[a // 2:b // 2, :], bf16)

    def phase1():
        h_ref[:, 0:PAD, :] = jnp.zeros((4, PAD, 128), f32)
        h_ref[:, PAD + S:PAD + S + PAD, :] = jnp.zeros((4, PAD, 128), f32)

        rep = jnp.where(_iota((32, 512), 0) == _iota((32, 512), 1) // 16, 1.0, 0.0).astype(bf16)
        lane_d = _iota((16, 512), 1) % 16
        low = _iota((8, 512), 0) < 4
        r = _iota((128, 128), 0)
        m2 = (r // 64) * 4 + r % 4 == _iota((128, 128), 1) // 16
        wait(g0)
        start(g6)
        w2d = wphi_ref[...].reshape(256, 32)
        cc = _nn(w2d, rep)
        e16 = cc[0:16, :]
        for d in range(1, DH):
            e16 = jnp.where(lane_d == d, cc[d * 16:(d + 1) * 16, :], e16)
        e64 = jnp.concatenate(
            [jnp.where(low, jnp.broadcast_to(e16[2 * i:2 * i + 1, :], (8, 512)),
                       jnp.broadcast_to(e16[2 * i + 1:2 * i + 2, :], (8, 512))) for i in range(8)], axis=0)
        et = jnp.concatenate([e64, e64], axis=0)
        bdt = jnp.where(jnp.concatenate([m2] * 4, axis=1), et, 0.0).astype(bf16)

        def fold(j, blocks):
            for b in blocks:
                lo = j * D + b * 128
                wt_ref[lo // 2:lo // 2 + 64, :] = pltpu.bitcast(
                    (_nt(bdt[:, b * 128:(b + 1) * 128], wqkv_ref[:, lo:lo + 128]) * LOG2E).astype(bf16), u32)

        def k_phi(kt):
            t = kt.shape[-1]
            ep, en, sp, sn = _exps(kt)
            phi = jnp.concatenate([(ep * (1.0 / sp)[None]).reshape(64, t),
                                   (en * (1.0 / sn)[None]).reshape(64, t)], axis=0)
            z = phi[:, 0:128]
            for c in range(1, t // 128):
                z = z + phi[:, c * 128:(c + 1) * 128]
            return phi, z

        def ln1(r0):
            _, xc, rs = _ln_stats(x_ref[r0:r0 + 128, :].astype(f32))
            return (xc * rs).astype(bf16)

        def h_rows(y, r0):
            h = _gelu(_nn(y, w1_ref[...]))
            for j in range(4):
                h_ref[j, PAD + r0:PAD + r0 + 128, :] = h[:, j * 128:(j + 1) * 128]

        phis = {}
        z_set = set()
        pending = []

        def feat(g, c, kt):
            phi, z = k_phi(kt)
            if g in z_set:
                z_ref[g] += z
            else:
                z_ref[g] = z
                z_set.add(g)
            for j in range(kt.shape[1] // 128):
                phis[(g, c + j * 128)] = phi[:, j * 128:(j + 1) * 128].astype(bf16)

        def kproj(g_lo, g_hi, c0, c1, defer=False):
            kt = _nt(wt(D + 64 * g_lo, D + 64 * g_hi), x_ref[c0:c1, :])
            n = c1 - c0
            for g in range(g_lo, g_hi):
                kg = kt[(g - g_lo) * 64:(g - g_lo + 1) * 64, :]
                if defer:
                    if n > 128:
                        feat(g, c0, kg[:, 0:n - 128])
                    pending.append((g, c1 - 128, kg[:, n - 128:n]))
                else:
                    feat(g, c0, kg)

        wait(g1)
        fold(1, [0, 1])
        wait(g2)
        kproj(0, 4, 0, 128, defer=True)
        wait(g3)
        fold(1, [2])
        kproj(0, 4, 128, 256)
        kproj(4, 6, 0, 256, defer=True)
        wait(g4)
        fold(1, [3])
        kproj(0, 6, 256, 512)
        kproj(6, 8, 0, 256)
        kproj(6, 8, 256, 512, defer=True)
        wait(g5)
        for p in pending:
            feat(*p)
        start(g7)
        wvt = wqkv_ref[:, 2 * D:3 * D].T
        wt_ref[D:3 * D // 2, :] = pltpu.bitcast(wvt, u32)
        kproj(0, G, 512, XC)
        vt = _nt(wvt, x_ref[0:XC, :])
        for g in range(G):
            acc = None
            for c in range(0, XC, 128):
                pr = _nt(vt[g * 64:(g + 1) * 64, c:c + 128].astype(bf16), phis[(g, c)])
                acc = pr if acc is None else acc + pr
            kv_ref[g] = acc
        y0 = ln1(0)
        wait(g6)

        h_rows(y0, 0)
        for i, r0 in enumerate(range(XC, S, TP)):
            if i == 1:
                fold(0, range(4))
            kvt = _nt(wt(D, 3 * D), x_ref[r0:r0 + TP, :])
            phs = []
            for g in range(G):
                phi, z = k_phi(kvt[g * 64:(g + 1) * 64, :])
                z_ref[g] += z
                phs.append(phi.astype(bf16))
            for g in range(G):
                kv_ref[g] += _nt(kvt[D + g * 64:D + (g + 1) * 64, :].astype(bf16), phs[g])
            for hr in (128 * (i + 1), r0, r0 + 128):
                h_rows(ln1(hr), hr)
        head_match = (_iota((64, 128), 0) // 16) == (_iota((64, 128), 1) % 4)
        for g in range(G):
            kvb_ref[g] = pltpu.bitcast(jnp.where(head_match, kv_ref[g], 0.0).astype(bf16), u32)
        wait(g7)

    def phase2(t):
        r0 = pl.multiple_of(t * T2, T2)
        x = x_ref[pl.ds(r0, T2), :]
        xf = x.astype(f32)
        gw = gw_ref[...].astype(f32).reshape(1, D)
        gate = 0.5 + 0.5 * jnp.tanh(0.5 * jnp.sum(xf * gw, axis=-1, keepdims=True))

        def mix(lo, hi):
            base = PAD + t * T2 + lo
            hs = jnp.concatenate([h_ref[j, pl.ds(base + off, hi - lo), :]
                                  for j, off in enumerate((-1, 1, -2, 2))], axis=1).astype(bf16)
            return xf[lo:hi, :] + _nn(hs, w2_ref[...])

        x1a = mix(0, 128)
        qt = _nt(wt(0, D), x)
        x1b = mix(128, T2 - 128)
        ots = []
        for g in range(G):
            ep, en, sp, sn = _exps(qt[g * 64:(g + 1) * 64, :])
            zb = jnp.broadcast_to(jnp.sum(z_ref[g], axis=-1, keepdims=True), (128, 128))
            z = jnp.concatenate([zb] * (T2 // 128), axis=1).reshape(16, 8, T2)
            dp = jnp.sum(ep * z[0:8], axis=0)
            dn = jnp.sum(en * z[8:16], axis=0)
            rr = 1.0 / (_fold4(dp * sn + dn * sp, jnp.add) + 1e-6 * (sp * sn))
            phi = jnp.concatenate([(ep * (sn * rr)[None]).reshape(64, T2),
                                   (en * (sp * rr)[None]).reshape(64, T2)], axis=0).astype(bf16)
            ots.append(_nn(pltpu.bitcast(kvb_ref[g], bf16), phi))
        ot = jnp.concatenate(ots, axis=0).astype(bf16)
        x1 = jnp.concatenate([x1a, x1b, mix(T2 - 128, T2)], axis=0)
        a = _tn(ot, wo_ref[...])
        m, _, rs = _ln_stats(x1)
        y = (x1 * rs - m * rs).astype(bf16)
        u = _gelu(_nt(y, w3t_ref[0:FM, :]))
        ut = _gelu(_nt(w3t_ref[FM:F, :], y)).astype(bf16).T
        c = x1 + gate * (a - x1)
        og = 1.0 - gate
        for j in range(4):
            sl = slice(j * 128, (j + 1) * 128)
            ra = 0
            for rn in ([T2] if j < 3 else [512, 256, 128, 128]):
                h2 = (_nn(u[ra:ra + rn, :].astype(bf16), w4_ref[0:FM, sl])
                      + _nn(ut[ra:ra + rn, :], w4_ref[FM:F, sl]))
                rows = pl.ds(pl.multiple_of(r0 + ra, 128), rn)
                o_ref[rows, sl] = (c[ra:ra + rn, sl] + og[ra:ra + rn] * h2).astype(bf16)
                cp(o_ref.at[rows, sl], o_hbm.at[rows, sl], sem.at[2]).start()
                ra += rn

    def step(t, carry):
        pl.when(t == 0)(phase1)
        pl.when(t > 0)(lambda: phase2(t - 1))
        return carry

    lax.fori_loop(0, 1 + S // T2, step, 0)
    cp(o_ref, o_hbm, sem.at[2]).wait()


@jax.jit
def pallas_gated_mix__linear_kernel_hedgehog__mixer_s_mlp__prompt_kernel(
    A_x: jax.Array,
    A_wqkv: jax.Array,
    A_w_phi: jax.Array,
    A_wo: jax.Array,
    B_x: jax.Array,
    B_w1: jax.Array,
    B_w2: jax.Array,
    B_w3: jax.Array,
    B_w4: jax.Array,
    gate_w: jax.Array,
):
    del B_x
    x = A_x.reshape(S, D)
    wphi = jnp.transpose(A_w_phi, (1, 2, 0))
    w3t = B_w3.T
    hbm = pl.BlockSpec(memory_space=pl.ANY)
    out = pl.pallas_call(
        _kernel,
        in_specs=[hbm] * 9,
        out_specs=hbm,
        out_shape=jax.ShapeDtypeStruct((S, D), bf16),
        scratch_shapes=[
            pltpu.VMEM((S, D), bf16),
            pltpu.VMEM((D, 3 * D), bf16),
            pltpu.VMEM((DH, DH, H), bf16),
            pltpu.VMEM((D, D), bf16),
            pltpu.VMEM((D, D), bf16),
            pltpu.VMEM((D, D), bf16),
            pltpu.VMEM((F, D), bf16),
            pltpu.VMEM((F, D), bf16),
            pltpu.VMEM((D,), bf16),
            pltpu.VMEM((S, D), bf16),
            pltpu.VMEM((3 * D // 2, D), u32),
            pltpu.VMEM((G, 64, 128), f32),
            pltpu.VMEM((G, 32, 128), u32),
            pltpu.VMEM((G, 128, 128), f32),
            pltpu.VMEM((4, S + 2 * PAD, 128), f32),
            pltpu.SemaphoreType.DMA((6,)),
        ],
        compiler_params=pltpu.CompilerParams(
            vmem_limit_bytes=100 * 1024 * 1024,
            disable_bounds_checks=True,
            disable_semaphore_checks=True,
        ),
    )(x, A_wqkv, wphi, A_wo, B_w1, B_w2, w3t, B_w4, gate_w)
    return out.reshape(1, S, D)
```

```python
import functools

import jax
import jax.numpy as jnp
from jax import lax
import jax.experimental.pallas as pl
import jax.experimental.pallas.tpu as pltpu

S, D, H, DH, F = 2048, 512, 32, 16, 1376
G = 8
FM = 1280
PAD = 8
T2 = 1024
XC = 768
HD, HF, HT = D // 2, FM // 2, T2 // 2
LOG2E = 1.4426950408889634

V0_ORDER = '5642713'
P1_SEQ = 'h6 v5 v2 v1 v3 h3 h4 h2 v4 h5 v7 h1 v6 h7'.split()
P2_SEQ = 'm5 q m3 m4 m1 m2 n m6 m7 o3 o1 o7 o2 o6 o4 o5 u4 u1 t u0 u2 u3'.split()
U_ORDERS = ('2357416', '1347526', '1743526', '4317256', '3546127')

f32 = jnp.float32
bf16 = jnp.bfloat16
u32 = jnp.uint32

_nn = functools.partial(jnp.dot, preferred_element_type=f32)
_nt = functools.partial(lax.dot_general, dimension_numbers=(((1,), (1,)), ((), ())),
                        preferred_element_type=f32)
_tn = functools.partial(lax.dot_general, dimension_numbers=(((0,), (0,)), ((), ())),
                        preferred_element_type=f32)


def _gelu(x):
    c = 0.7978845608028654
    inner = x * (c + (c * 0.044715) * (x * x))
    hx = 0.5 * x
    return hx + hx * jnp.tanh(inner)


def _ln_stats(x):
    m = jnp.mean(x, axis=-1, keepdims=True)
    xc = x - m
    v = jnp.mean(xc * xc, axis=-1, keepdims=True)
    return m, xc, lax.rsqrt(v + 1e-5)


def _fold4(v, op):
    return op(v, pltpu.roll(v, 4, 0))


def _exps(p):
    p3 = p.reshape(8, 8, p.shape[-1])
    mx = _fold4(jnp.max(p3, axis=0), jnp.maximum)
    mn = _fold4(jnp.min(p3, axis=0), jnp.minimum)
    ep = jnp.exp2(p3 - mx[None])
    en = jnp.exp2(mn[None] - p3)
    sp = _fold4(jnp.sum(ep, axis=0), jnp.add)
    sn = _fold4(jnp.sum(en, axis=0), jnp.add)
    return ep, en, sp, sn


def _left_ops(a11, a12, a21, a22):
    return [v.astype(bf16) for v in
            (a11 + a22, a21 + a22, a11, a22, a11 + a12, a21 - a11, a12 - a22)]


def _right_ops(read):
    f = lambda i, k: read(i, k).astype(f32)
    return [(f(0, 0) + f(3, 0)).astype(bf16), read(0, 1), (f(1, 2) - f(3, 2)).astype(bf16),
            (f(2, 3) - f(0, 3)).astype(bf16), read(3, 4), (f(0, 5) + f(1, 5)).astype(bf16),
            (f(2, 6) + f(3, 6)).astype(bf16)]


def _combine(m, order):
    pos = {int(k): i for i, k in enumerate(order)}

    def comb(terms):
        terms = sorted(terms, key=lambda t: pos[abs(t)])
        if terms[0] < 0:
            acc, rest = m[terms[1]] - m[-terms[0]], terms[2:]
        else:
            acc, rest = m[terms[0]], terms[1:]
        for t in rest:
            acc = acc + m[t] if t > 0 else acc - m[-t]
        return acc

    return comb([1, 4, -5, 7]), comb([3, 5]), comb([2, 4]), comb([1, -2, 3, 6])


def _strassen(mm, a, b, order):
    m = {}
    for k in order:
        m[int(k)] = mm(a[int(k) - 1], b[int(k) - 1])
    return _combine(m, order)


def _quad(v):
    r, c = v.shape[0] // 2, v.shape[1] // 2
    return v[0:r, 0:c], v[0:r, c:], v[r:, 0:c], v[r:, c:]


def _join(c11, c12, c21, c22):
    return jnp.concatenate([jnp.concatenate([c11, c12], axis=1),
                            jnp.concatenate([c21, c22], axis=1)], axis=0)


def _iota(shape, dim):
    return lax.broadcasted_iota(jnp.int32, shape, dim)


def _kernel(x_hbm, wqkv_hbm, wphi_hbm, wo_hbm, w1_hbm, w2_hbm, w3t_hbm, w4_hbm, gw_hbm, o_hbm,
            x_ref, wqkv_ref, wphi_ref, wo_ref, w1_ref, w2_ref, w3t_ref, w4_ref, gw_ref, o_ref,
            wq_ref, kv_ref, kvb_ref, z_ref, h_ref, sem):
    cp = pltpu.make_async_copy
    lo_, hi_ = slice(0, HD), slice(HD, D)

    def w_cols(a, b, s):
        return cp(wqkv_hbm.at[:, a:b], wqkv_ref.at[:, a:b], sem.at[s])

    def x_rows(a, b, s):
        return cp(x_hbm.at[a:b, :], x_ref.at[a:b, :], sem.at[s])

    def start(cs):
        for c in cs:
            c.start()

    def wait(cs):
        for c in cs:
            c.wait()

    g0 = [cp(wphi_hbm, wphi_ref, sem.at[0])]
    g1 = [w_cols(D, D + 256, 1)]
    g2 = [x_rows(0, 128, 2)]
    g3 = [w_cols(D + 256, D + 384, 3), x_rows(128, 256, 3)]
    g4 = [w_cols(D + 384, 2 * D, 4), x_rows(256, 512, 4)]
    g5 = [w_cols(2 * D, 3 * D, 5), x_rows(512, XC, 5), cp(gw_hbm, gw_ref, sem.at[5])]
    g6 = [cp(w1_hbm, w1_ref, sem.at[0]), x_rows(XC, S, 0), w_cols(0, D, 0)]
    g7 = [cp(w2_hbm, w2_ref, sem.at[1]), cp(wo_hbm, wo_ref, sem.at[1]),
          cp(w3t_hbm, w3t_ref, sem.at[1]), cp(w4_hbm, w4_ref, sem.at[1])]
    start(g0 + g1 + g2 + g3 + g4 + g5)

    def right_ops(t, ref, blocks):
        def read(i, k):
            r, n, cols = blocks[i]
            return ref[pl.ds(pl.multiple_of((t >> (2 + k)) * 16 + r, 16), n), cols]
        return _right_ops(read)

    def phase1(t):
        h_ref[:, 0:PAD, :] = jnp.zeros((4, PAD, 128), f32)
        h_ref[:, PAD + S:PAD + S + PAD, :] = jnp.zeros((4, PAD, 128), f32)

        rep = jnp.where(_iota((32, 512), 0) == _iota((32, 512), 1) // 16, 1.0, 0.0).astype(bf16)
        lane_d = _iota((16, 512), 1) % 16
        low = _iota((8, 512), 0) < 4
        r = _iota((128, 128), 0)
        m2 = (r // 64) * 4 + r % 4 == _iota((128, 128), 1) // 16
        wait(g0)
        start(g6)
        w2d = wphi_ref[...].reshape(256, 32)
        cc = _nn(w2d, rep)
        e16 = cc[0:16, :]
        for d in range(1, DH):
            e16 = jnp.where(lane_d == d, cc[d * 16:(d + 1) * 16, :], e16)
        e64 = jnp.concatenate(
            [jnp.where(low, jnp.broadcast_to(e16[2 * i:2 * i + 1, :], (8, 512)),
                       jnp.broadcast_to(e16[2 * i + 1:2 * i + 2, :], (8, 512))) for i in range(8)], axis=0)
        et = jnp.concatenate([e64, e64], axis=0)
        bdt = jnp.where(jnp.concatenate([m2] * 4, axis=1), et, 0.0).astype(bf16)

        def fold(c0, b):
            lo = c0 + b * 128
            return _nt(bdt[:, b * 128:(b + 1) * 128], wqkv_ref[:, lo:lo + 128]) * LOG2E

        def k_phi(kt):
            n = kt.shape[-1]
            ep, en, sp, sn = _exps(kt)
            phi = jnp.concatenate([(ep * (1.0 / sp)[None]).reshape(64, n),
                                   (en * (1.0 / sn)[None]).reshape(64, n)], axis=0)
            z = phi[:, 0:128]
            for c in range(1, n // 128):
                z = z + phi[:, c * 128:(c + 1) * 128]
            return phi, z

        def x_ops(c0, c1):
            n = (c1 - c0) // 2
            return right_ops(t, x_ref, [(c0, n, lo_), (c0 + n, n, lo_), (c0, n, hi_), (c0 + n, n, hi_)])

        wk = {}
        phis = {}
        z_set = set()
        pending = []

        def feat(g, c, kt):
            phi, z = k_phi(kt)
            if g in z_set:
                z_ref[g] += z
            else:
                z_ref[g] = z
                z_set.add(g)
            for j in range(kt.shape[1] // 128):
                phis[(g, c + j * 128)] = phi[:, j * 128:(j + 1) * 128].astype(bf16)

        def kproj(g_lo, g_hi, c0, c1, defer=False):
            w = jnp.concatenate([wk[b] for b in range(g_lo // 2, g_hi // 2)], axis=0)
            kt = _nt(w.astype(bf16), x_ref[c0:c1, :])
            n = c1 - c0
            for g in range(g_lo, g_hi):
                kg = kt[(g - g_lo) * 64:(g - g_lo + 1) * 64, :]
                if defer:
                    if n > 128:
                        feat(g, c0, kg[:, 0:n - 128])
                    pending.append((g, c1 - 128, kg[:, n - 128:n]))
                else:
                    feat(g, c0, kg)

        wait(g1)
        wk[0] = fold(D, 0)
        wk[1] = fold(D, 1)
        wait(g2)
        kproj(0, 4, 0, 128, defer=True)
        wait(g3)
        wk[2] = fold(D, 2)
        kproj(0, 4, 128, 256)
        kproj(4, 6, 0, 256, defer=True)
        wait(g4)
        wk[3] = fold(D, 3)
        kproj(0, 6, 256, 512)
        kproj(6, 8, 0, 256)
        kproj(6, 8, 256, 512, defer=True)
        wait(g5)
        for p in pending:
            feat(*p)
        start(g7)
        wvq = _quad(wqkv_ref[:, 2 * D:3 * D].T.astype(f32))
        wva = _left_ops(*wvq)
        kproj(0, G, 512, XC)
        vt = _join(*_strassen(_nt, wva, x_ops(0, XC), V0_ORDER))
        for g in range(G):
            acc = None
            for c in range(0, XC, 128):
                pr = _nt(vt[g * 64:(g + 1) * 64, c:c + 128].astype(bf16), phis[(g, c)])
                acc = pr if acc is None else acc + pr
            kv_ref[g] = acc
        wait(g6)

        wkq = _quad(jnp.concatenate([wk[b] for b in range(4)], axis=0))
        kva = _left_ops(*[jnp.concatenate([a, b], axis=0) for a, b in zip(wkq, wvq)])
        w1q = _quad(w1_ref[...])
        hb = _right_ops(lambda i, k: w1q[i])
        ys = []
        for r0 in (0, S // 2):
            _, xc, rs = _ln_stats(x_ref[r0:r0 + S // 2, :].astype(f32))
            ys.append(xc * rs)
        ha = _left_ops(ys[0][:, lo_], ys[0][:, hi_], ys[1][:, lo_], ys[1][:, hi_])
        xb = x_ops(XC, S)
        vm, hm = {}, {}
        for op in P1_SEQ:
            k = int(op[1])
            if op[0] == 'v':
                vm[k] = _nt(kva[k - 1], xb[k - 1])
            else:
                hm[k] = _nn(ha[k - 1], hb[k - 1])
        for i, c in enumerate(_combine(hm, [op[1] for op in P1_SEQ if op[0] == 'h'])):
            h = _gelu(c)
            r0 = PAD + (i // 2) * (S // 2)
            for j in range(2):
                h_ref[(i % 2) * 2 + j, r0:r0 + S // 2, :] = h[:, j * 128:(j + 1) * 128]
        for b in range(4):
            wq_ref[b * 64:(b + 1) * 64, :] = pltpu.bitcast(fold(0, b).astype(bf16), u32)
        cs = _combine(vm, [op[1] for op in P1_SEQ if op[0] == 'v'])
        kt = _join(*[c[0:HD] for c in cs])
        vt = _join(*[c[HD:D] for c in cs])
        phs = []
        for g in range(G):
            phi, z = k_phi(kt[g * 64:(g + 1) * 64, :])
            z_ref[g] += z
            phs.append(phi.astype(bf16))
        for g in range(G):
            kv_ref[g] += _nt(vt[g * 64:(g + 1) * 64, :].astype(bf16), phs[g])
        head_match = (_iota((64, 128), 0) // 16) == (_iota((64, 128), 1) % 4)
        for g in range(G):
            kvb_ref[g] = pltpu.bitcast(jnp.where(head_match, kv_ref[g], 0.0).astype(bf16), u32)
        wait(g7)

    def phase2(t):
        r0 = pl.multiple_of(t * T2, T2)
        x = x_ref[pl.ds(r0, T2), :]
        xf = x.astype(f32)
        gw = gw_ref[...].astype(f32).reshape(1, D)
        xg = x_ref[pl.ds(pl.multiple_of(r0 + (t >> 2) * 16, 16), T2), :].astype(f32)
        gate = 0.5 + 0.5 * jnp.tanh(0.5 * jnp.sum(xg * gw, axis=-1, keepdims=True))

        square = [(0, HD, lo_), (0, HD, hi_), (HD, HD, lo_), (HD, HD, hi_)]
        base = PAD + t * T2
        hs = jnp.concatenate([h_ref[j, pl.ds(base + off, T2), :]
                              for j, off in enumerate((-1, 1, -2, 2))], axis=1)
        ha = _left_ops(*_quad(hs))
        hb = right_ops(t, w2_ref, square)
        ob = right_ops(t, wo_ref, square)
        mm, om, us, st = {}, {}, {}, {}

        def norm2():
            if 'y' not in st:
                x1 = xf + _join(*_combine(mm, [op[1] for op in P2_SEQ if op[0] == 'm']))
                m, _, rs = _ln_stats(x1)
                yf = x1 * rs - m * rs
                st['x1'], st['y'], st['ya'] = x1, yf.astype(bf16), _left_ops(*_quad(yf))
            return st

        for op in P2_SEQ:
            if op == 'q':
                qt = _nt(pltpu.bitcast(wq_ref[...], bf16), x)
            elif op == 'n':
                ots = []
                for g in range(G):
                    ep, en, sp, sn = _exps(qt[g * 64:(g + 1) * 64, :])
                    zb = jnp.broadcast_to(jnp.sum(z_ref[g], axis=-1, keepdims=True), (128, 128))
                    z = jnp.concatenate([zb] * (T2 // 128), axis=1).reshape(16, 8, T2)
                    dp = jnp.sum(ep * z[0:8], axis=0)
                    dn = jnp.sum(en * z[8:16], axis=0)
                    rr = 1.0 / (_fold4(dp * sn + dn * sp, jnp.add) + 1e-6 * (sp * sn))
                    phi = jnp.concatenate([(ep * (sn * rr)[None]).reshape(64, T2),
                                           (en * (sp * rr)[None]).reshape(64, T2)], axis=0).astype(bf16)
                    ots.append(_nn(pltpu.bitcast(kvb_ref[g], bf16), phi))
                t11, t21, t12, t22 = _quad(jnp.concatenate(ots, axis=0))
                oa = _left_ops(t11, t12, t21, t22)
            elif op == 't':
                ut = _gelu(_nt(w3t_ref[FM:F, :], norm2()['y'])).astype(bf16).T
            elif op[0] == 'm':
                k = int(op[1])
                mm[k] = _nn(ha[k - 1], hb[k - 1])
            elif op[0] == 'o':
                k = int(op[1])
                om[k] = _tn(oa[k - 1], ob[k - 1])
            elif op[0] == 'u':
                j = int(op[1])
                n0 = j * 128
                ub = right_ops(t, w3t_ref, [(n0, 128, lo_), (HF + n0, 128, lo_),
                                            (n0, 128, hi_), (HF + n0, 128, hi_)])
                us[j] = [_gelu(v) for v in _strassen(_nt, norm2()['ya'], ub, U_ORDERS[j])]
        a = _join(*_combine(om, [op[1] for op in P2_SEQ if op[0] == 'o']))
        x1 = st['x1']
        ua = _left_ops(*[jnp.concatenate([us[j][i] for j in range(5)], axis=1) for i in range(4)])

        def emit(ra, rn, c0, h2):
            cols = slice(c0, c0 + 128)
            rows = pl.ds(pl.multiple_of(r0 + ra, 128), rn)
            b = x1[ra:ra + rn, cols] + h2
            o_ref[rows, cols] = (b + gate[ra:ra + rn] * (a[ra:ra + rn, cols] - b)).astype(bf16)
            cp(o_ref.at[rows, cols], o_hbm.at[rows, cols], sem.at[2]).start()

        for n0 in (0, 128):
            cl, cr = slice(n0, n0 + 128), slice(HD + n0, HD + n0 + 128)
            wb = right_ops(t, w4_ref, [(0, HF, cl), (0, HF, cr), (HF, HF, cl), (HF, HF, cr)])
            tl, tr = w4_ref[FM:F, cl], w4_ref[FM:F, cr]
            prod = lambda k, rs=slice(0, HT): _nn(ua[k - 1][rs], wb[k - 1])
            m3 = prod(3)
            m5 = prod(5)
            emit(0, HT, HD + n0, (m3 + m5) + _nn(ut[0:HT], tr))
            m4 = prod(4)
            m2 = prod(2)
            emit(HT, HT, n0, (m4 + m2) + _nn(ut[HT:T2], tl))
            m1 = prod(1)
            emit(0, HT, n0, ((m4 - m5) + m1) + prod(7) + _nn(ut[0:HT], tl))
            p22 = (m3 - m2) + m1
            ra = 0
            for rn in ([HT] if n0 == 0 else [256, 128, 128]):
                rs = slice(ra, ra + rn)
                emit(HT + ra, rn, HD + n0, p22[rs] + prod(6, rs) + _nn(ut[HT + ra:HT + ra + rn], tr))
                ra += rn

    def step(t, carry):
        pl.when(t == 0)(lambda: phase1(t))
        pl.when(t > 0)(lambda: phase2(t - 1))
        return carry

    lax.fori_loop(0, 1 + S // T2, step, 0)
    cp(o_ref, o_hbm, sem.at[2]).wait()


@jax.jit
def pallas_gated_mix__linear_kernel_hedgehog__mixer_s_mlp__prompt_kernel(
    A_x: jax.Array,
    A_wqkv: jax.Array,
    A_w_phi: jax.Array,
    A_wo: jax.Array,
    B_x: jax.Array,
    B_w1: jax.Array,
    B_w2: jax.Array,
    B_w3: jax.Array,
    B_w4: jax.Array,
    gate_w: jax.Array,
):
    del B_x
    x = A_x.reshape(S, D)
    wphi = jnp.transpose(A_w_phi, (1, 2, 0))
    w3t = B_w3.T
    hbm = pl.BlockSpec(memory_space=pl.ANY)
    out = pl.pallas_call(
        _kernel,
        in_specs=[hbm] * 9,
        out_specs=hbm,
        out_shape=jax.ShapeDtypeStruct((S, D), bf16),
        scratch_shapes=[
            pltpu.VMEM((S, D), bf16),
            pltpu.VMEM((D, 3 * D), bf16),
            pltpu.VMEM((DH, DH, H), bf16),
            pltpu.VMEM((D, D), bf16),
            pltpu.VMEM((D, D), bf16),
            pltpu.VMEM((D, D), bf16),
            pltpu.VMEM((F, D), bf16),
            pltpu.VMEM((F, D), bf16),
            pltpu.VMEM((D,), bf16),
            pltpu.VMEM((S, D), bf16),
            pltpu.VMEM((D // 2, D), u32),
            pltpu.VMEM((G, 64, 128), f32),
            pltpu.VMEM((G, 32, 128), u32),
            pltpu.VMEM((G, 128, 128), f32),
            pltpu.VMEM((4, S + 2 * PAD, 128), f32),
            pltpu.SemaphoreType.DMA((6,)),
        ],
        compiler_params=pltpu.CompilerParams(
            vmem_limit_bytes=100 * 1024 * 1024,
            disable_bounds_checks=True,
            disable_semaphore_checks=True,
        ),
    )(x, A_wqkv, wphi, A_wo, B_w1, B_w2, w3t, B_w4, gate_w)
    return out.reshape(1, S, D)
```

```python
import functools

import jax
import jax.numpy as jnp
from jax import lax
import jax.experimental.pallas as pl
import jax.experimental.pallas.tpu as pltpu

S, D, H, DH, F = 2048, 512, 32, 16, 1376
G = 8
FM = 1280
PAD = 8
T2 = 1024
XC = 768
HD, HF, HT = D // 2, FM // 2, T2 // 2
LOG2E = 1.4426950408889634

V0_ORDER = '5642713'
P1_SEQ = 'h6 v5 v2 v1 v3 h3 h4 h2 v4 h5 v7 h1 v6 h7'.split()
P2_SEQ = 'm5 q m3 m4 m1 m2 n m6 m7 o3 o1 o7 o2 o6 o4 o5 u4 u1 t u0 u2 u3'.split()
U_ORDERS = ('2357416', '1347526', '1743526', '4317256', '3546127')

f32 = jnp.float32
bf16 = jnp.bfloat16
u32 = jnp.uint32

_nn = functools.partial(jnp.dot, preferred_element_type=f32)
_nt = functools.partial(lax.dot_general, dimension_numbers=(((1,), (1,)), ((), ())),
                        preferred_element_type=f32)
_tn = functools.partial(lax.dot_general, dimension_numbers=(((0,), (0,)), ((), ())),
                        preferred_element_type=f32)


def _gelu(x):
    c = 0.7978845608028654
    inner = x * (c + (c * 0.044715) * (x * x))
    hx = 0.5 * x
    return hx + hx * jnp.tanh(inner)


def _ln_stats(x):
    m = jnp.mean(x, axis=-1, keepdims=True)
    xc = x - m
    v = jnp.mean(xc * xc, axis=-1, keepdims=True)
    return m, xc, lax.rsqrt(v + 1e-5)


def _fold4(v, op):
    return op(v, pltpu.roll(v, 4, 0))


def _exps(p):
    p3 = p.reshape(8, 8, p.shape[-1])
    mx = _fold4(jnp.max(p3, axis=0), jnp.maximum)
    mn = _fold4(jnp.min(p3, axis=0), jnp.minimum)
    ep = jnp.exp2(p3 - mx[None])
    en = jnp.exp2(mn[None] - p3)
    sp = _fold4(jnp.sum(ep, axis=0), jnp.add)
    sn = _fold4(jnp.sum(en, axis=0), jnp.add)
    return ep, en, sp, sn


def _left_ops(a11, a12, a21, a22):
    return [v.astype(bf16) for v in
            (a11 + a22, a21 + a22, a11, a22, a11 + a12, a21 - a11, a12 - a22)]


def _right_ops(read):
    f = lambda i, k: read(i, k).astype(f32)
    return [(f(0, 0) + f(3, 0)).astype(bf16), read(0, 1), (f(1, 2) - f(3, 2)).astype(bf16),
            (f(2, 3) - f(0, 3)).astype(bf16), read(3, 4), (f(0, 5) + f(1, 5)).astype(bf16),
            (f(2, 6) + f(3, 6)).astype(bf16)]


def _combine(m, order):
    pos = {int(k): i for i, k in enumerate(order)}

    def comb(terms):
        terms = sorted(terms, key=lambda t: pos[abs(t)])
        if terms[0] < 0:
            acc, rest = m[terms[1]] - m[-terms[0]], terms[2:]
        else:
            acc, rest = m[terms[0]], terms[1:]
        for t in rest:
            acc = acc + m[t] if t > 0 else acc - m[-t]
        return acc

    return comb([1, 4, -5, 7]), comb([3, 5]), comb([2, 4]), comb([1, -2, 3, 6])


def _strassen(mm, a, b, order):
    m = {}
    for k in order:
        m[int(k)] = mm(a[int(k) - 1], b[int(k) - 1])
    return _combine(m, order)


def _quad(v):
    r, c = v.shape[0] // 2, v.shape[1] // 2
    return v[0:r, 0:c], v[0:r, c:], v[r:, 0:c], v[r:, c:]


def _join(c11, c12, c21, c22):
    return jnp.concatenate([jnp.concatenate([c11, c12], axis=1),
                            jnp.concatenate([c21, c22], axis=1)], axis=0)


def _iota(shape, dim):
    return lax.broadcasted_iota(jnp.int32, shape, dim)


def _kernel(x_hbm, wqkv_hbm, wphi_hbm, wo_hbm, w1_hbm, w2_hbm, w3t_hbm, w4_hbm, gw_hbm, o_hbm,
            x_ref, wqkv_ref, wphi_ref, wo_ref, w1_ref, w2_ref, w3t_ref, w4_ref, gw_ref, o_ref,
            wq_ref, kv_ref, kvb_ref, z_ref, h_ref, sem):
    cp = pltpu.make_async_copy
    lo_, hi_ = slice(0, HD), slice(HD, D)

    def w_cols(a, b, s):
        return cp(wqkv_hbm.at[:, a:b], wqkv_ref.at[:, a:b], sem.at[s])

    def x_rows(a, b, s):
        return cp(x_hbm.at[a:b, :], x_ref.at[a:b, :], sem.at[s])

    def start(cs):
        for c in cs:
            c.start()

    def wait(cs):
        for c in cs:
            c.wait()

    g0 = [cp(wphi_hbm, wphi_ref, sem.at[0])]
    g1 = [w_cols(D, D + 256, 1)]
    g2 = [x_rows(0, 128, 2)]
    g3 = [w_cols(D + 256, D + 384, 3), x_rows(128, 256, 3)]
    g4 = [w_cols(D + 384, 2 * D, 4), x_rows(256, 512, 4)]
    g5 = [w_cols(2 * D, 3 * D, 5), x_rows(512, XC, 5), cp(gw_hbm, gw_ref, sem.at[5])]
    g6 = [cp(w1_hbm, w1_ref, sem.at[0]), x_rows(XC, S, 0), w_cols(0, D, 0)]
    g7 = [cp(w2_hbm, w2_ref, sem.at[1]), cp(wo_hbm, wo_ref, sem.at[1]),
          cp(w3t_hbm, w3t_ref, sem.at[1]), cp(w4_hbm, w4_ref, sem.at[1])]
    start(g0 + g1 + g2 + g3 + g4 + g5)

    def right_ops(t, ref, blocks):
        def read(i, k):
            r, n, cols = blocks[i]
            return ref[pl.ds(pl.multiple_of((t >> (2 + k)) * 16 + r, 16), n), cols]
        return _right_ops(read)

    def phase1(t):
        h_ref[:, PAD:2 * PAD, :] = jnp.zeros((4, PAD, 128), f32)
        h_ref[:, S:PAD + S, :] = jnp.zeros((4, PAD, 128), f32)

        rep = jnp.where(_iota((32, 512), 0) == _iota((32, 512), 1) // 16, 1.0, 0.0).astype(bf16)
        lane_d = _iota((16, 512), 1) % 16
        low = _iota((8, 512), 0) < 4
        r = _iota((128, 128), 0)
        m2 = (r // 64) * 4 + r % 4 == _iota((128, 128), 1) // 16
        wait(g0)
        start(g6)
        w2d = wphi_ref[...].reshape(256, 32)
        cc = _nn(w2d, rep)
        e16 = cc[0:16, :]
        for d in range(1, DH):
            e16 = jnp.where(lane_d == d, cc[d * 16:(d + 1) * 16, :], e16)
        e64 = jnp.concatenate(
            [jnp.where(low, jnp.broadcast_to(e16[2 * i:2 * i + 1, :], (8, 512)),
                       jnp.broadcast_to(e16[2 * i + 1:2 * i + 2, :], (8, 512))) for i in range(8)], axis=0)
        et = jnp.concatenate([e64, e64], axis=0)
        bdt = jnp.where(jnp.concatenate([m2] * 4, axis=1), et, 0.0).astype(bf16)

        def fold(c0, b):
            lo = c0 + b * 128
            return _nt(bdt[:, b * 128:(b + 1) * 128], wqkv_ref[:, lo:lo + 128]) * LOG2E

        def k_phi(kt):
            n = kt.shape[-1]
            ep, en, sp, sn = _exps(kt)
            phi = jnp.concatenate([(ep * (1.0 / sp)[None]).reshape(64, n),
                                   (en * (1.0 / sn)[None]).reshape(64, n)], axis=0)
            z = phi[:, 0:128]
            for c in range(1, n // 128):
                z = z + phi[:, c * 128:(c + 1) * 128]
            return phi, z

        def x_ops(c0, c1):
            n = (c1 - c0) // 2
            return right_ops(t, x_ref, [(c0, n, lo_), (c0 + n, n, lo_), (c0, n, hi_), (c0 + n, n, hi_)])

        wk = {}
        phis = {}
        z_set = set()
        pending = []

        def feat(g, c, kt):
            phi, z = k_phi(kt)
            if g in z_set:
                z_ref[g] += z
            else:
                z_ref[g] = z
                z_set.add(g)
            for j in range(kt.shape[1] // 128):
                phis[(g, c + j * 128)] = phi[:, j * 128:(j + 1) * 128].astype(bf16)

        def kproj(g_lo, g_hi, c0, c1, defer=False):
            w = jnp.concatenate([wk[b] for b in range(g_lo // 2, g_hi // 2)], axis=0)
            kt = _nt(w.astype(bf16), x_ref[c0:c1, :])
            n = c1 - c0
            for g in range(g_lo, g_hi):
                kg = kt[(g - g_lo) * 64:(g - g_lo + 1) * 64, :]
                if defer:
                    if n > 128:
                        feat(g, c0, kg[:, 0:n - 128])
                    pending.append((g, c1 - 128, kg[:, n - 128:n]))
                else:
                    feat(g, c0, kg)

        wait(g1)
        wk[0] = fold(D, 0)
        wk[1] = fold(D, 1)
        wait(g2)
        kproj(0, 4, 0, 128, defer=True)
        wait(g3)
        wk[2] = fold(D, 2)
        kproj(0, 4, 128, 256)
        kproj(4, 6, 0, 256, defer=True)
        wait(g4)
        wk[3] = fold(D, 3)
        kproj(0, 6, 256, 512)
        kproj(6, 8, 0, 256)
        kproj(6, 8, 256, 512, defer=True)
        wait(g5)
        for p in pending:
            feat(*p)
        start(g7)
        wvq = _quad(wqkv_ref[:, 2 * D:3 * D].T.astype(f32))
        wva = _left_ops(*wvq)
        kproj(0, G, 512, XC)
        vt = _join(*_strassen(_nt, wva, x_ops(0, XC), V0_ORDER))
        for g in range(G):
            acc = None
            for c in range(0, XC, 128):
                pr = _nt(vt[g * 64:(g + 1) * 64, c:c + 128].astype(bf16), phis[(g, c)])
                acc = pr if acc is None else acc + pr
            kv_ref[g] = acc
        wait(g6)

        wkq = _quad(jnp.concatenate([wk[b] for b in range(4)], axis=0))
        kva = _left_ops(*[jnp.concatenate([a, b], axis=0) for a, b in zip(wkq, wvq)])
        w1q = _quad(w1_ref[...])
        hb = _right_ops(lambda i, k: w1q[i])
        ys = []
        for r0 in (0, S // 2):
            _, xc, rs = _ln_stats(x_ref[r0:r0 + S // 2, :].astype(f32))
            ys.append(xc * rs)
        ha = _left_ops(ys[0][:, lo_], ys[0][:, hi_], ys[1][:, lo_], ys[1][:, hi_])
        xb = x_ops(XC, S)
        vm, hm = {}, {}
        for op in P1_SEQ:
            k = int(op[1])
            if op[0] == 'v':
                vm[k] = _nt(kva[k - 1], xb[k - 1])
            else:
                hm[k] = _nn(ha[k - 1], hb[k - 1])
        for i, c in enumerate(_combine(hm, [op[1] for op in P1_SEQ if op[0] == 'h'])):
            h = _gelu(c)
            r0 = PAD + (i // 2) * (S // 2)
            for j in range(2):
                ch = (i % 2) * 2 + j
                rs = r0 + (1, -1, 2, -2)[ch]
                h_ref[ch, rs:rs + S // 2, :] = h[:, j * 128:(j + 1) * 128]
        for b in range(4):
            wq_ref[b * 64:(b + 1) * 64, :] = pltpu.bitcast(fold(0, b).astype(bf16), u32)
        cs = _combine(vm, [op[1] for op in P1_SEQ if op[0] == 'v'])
        kt = _join(*[c[0:HD] for c in cs])
        vt = _join(*[c[HD:D] for c in cs])
        phs = []
        for g in range(G):
            phi, z = k_phi(kt[g * 64:(g + 1) * 64, :])
            z_ref[g] += z
            phs.append(phi.astype(bf16))
        for g in range(G):
            kv_ref[g] += _nt(vt[g * 64:(g + 1) * 64, :].astype(bf16), phs[g])
        head_match = (_iota((64, 128), 0) // 16) == (_iota((64, 128), 1) % 4)
        for g in range(G):
            kvb_ref[g] = pltpu.bitcast(jnp.where(head_match, kv_ref[g], 0.0).astype(bf16), u32)
        wait(g7)

    def phase2(t):
        r0 = pl.multiple_of(t * T2, T2)
        x = x_ref[pl.ds(r0, T2), :]
        xf = x.astype(f32)
        gw = gw_ref[...].astype(f32).reshape(1, D)
        xg = x_ref[pl.ds(pl.multiple_of(r0 + (t >> 2) * 16, 16), T2), :].astype(f32)
        gate = 0.5 + 0.5 * jnp.tanh(0.5 * jnp.sum(xg * gw, axis=-1, keepdims=True))

        square = [(0, HD, lo_), (0, HD, hi_), (HD, HD, lo_), (HD, HD, hi_)]
        base = pl.multiple_of(PAD + t * T2, 8)
        hs = jnp.concatenate([h_ref[j, pl.ds(base, T2), :] for j in range(4)], axis=1)
        ha = _left_ops(*_quad(hs))
        hb = right_ops(t, w2_ref, square)
        ob = right_ops(t, wo_ref, square)
        mm, om, us, st = {}, {}, {}, {}

        def norm2():
            if 'y' not in st:
                x1 = xf + _join(*_combine(mm, [op[1] for op in P2_SEQ if op[0] == 'm']))
                m, _, rs = _ln_stats(x1)
                yf = x1 * rs - m * rs
                st['x1'], st['y'], st['ya'] = x1, yf.astype(bf16), _left_ops(*_quad(yf))
            return st

        for op in P2_SEQ:
            if op == 'q':
                qt = _nt(pltpu.bitcast(wq_ref[...], bf16), x)
            elif op == 'n':
                ots = []
                for g in range(G):
                    ep, en, sp, sn = _exps(qt[g * 64:(g + 1) * 64, :])
                    zb = jnp.broadcast_to(jnp.sum(z_ref[g], axis=-1, keepdims=True), (128, 128))
                    z = jnp.concatenate([zb] * (T2 // 128), axis=1).reshape(16, 8, T2)
                    dp = jnp.sum(ep * z[0:8], axis=0)
                    dn = jnp.sum(en * z[8:16], axis=0)
                    rr = 1.0 / (_fold4(dp * sn + dn * sp, jnp.add) + 1e-6 * (sp * sn))
                    phi = jnp.concatenate([(ep * (sn * rr)[None]).reshape(64, T2),
                                           (en * (sp * rr)[None]).reshape(64, T2)], axis=0).astype(bf16)
                    ots.append(_nn(pltpu.bitcast(kvb_ref[g], bf16), phi))
                t11, t21, t12, t22 = _quad(jnp.concatenate(ots, axis=0))
                oa = _left_ops(t11, t12, t21, t22)
            elif op == 't':
                ut = _gelu(_nt(w3t_ref[FM:F, :], norm2()['y'])).astype(bf16).T
            elif op[0] == 'm':
                k = int(op[1])
                mm[k] = _nn(ha[k - 1], hb[k - 1])
            elif op[0] == 'o':
                k = int(op[1])
                om[k] = _tn(oa[k - 1], ob[k - 1])
            elif op[0] == 'u':
                j = int(op[1])
                n0 = j * 128
                ub = right_ops(t, w3t_ref, [(n0, 128, lo_), (HF + n0, 128, lo_),
                                            (n0, 128, hi_), (HF + n0, 128, hi_)])
                us[j] = [_gelu(v) for v in _strassen(_nt, norm2()['ya'], ub, U_ORDERS[j])]
        a = _join(*_combine(om, [op[1] for op in P2_SEQ if op[0] == 'o']))
        x1 = st['x1']
        ua = _left_ops(*[jnp.concatenate([us[j][i] for j in range(5)], axis=1) for i in range(4)])

        def emit(ra, rn, c0, h2):
            cols = slice(c0, c0 + 128)
            rows = pl.ds(pl.multiple_of(r0 + ra, 128), rn)
            b = x1[ra:ra + rn, cols] + h2
            o_ref[rows, cols] = (b + gate[ra:ra + rn] * (a[ra:ra + rn, cols] - b)).astype(bf16)
            cp(o_ref.at[rows, cols], o_hbm.at[rows, cols], sem.at[2]).start()

        for n0 in (0, 128):
            cl, cr = slice(n0, n0 + 128), slice(HD + n0, HD + n0 + 128)
            wb = right_ops(t, w4_ref, [(0, HF, cl), (0, HF, cr), (HF, HF, cl), (HF, HF, cr)])
            tl, tr = w4_ref[FM:F, cl], w4_ref[FM:F, cr]
            prod = lambda k, rs=slice(0, HT): _nn(ua[k - 1][rs], wb[k - 1])
            m3 = prod(3)
            m5 = prod(5)
            emit(0, HT, HD + n0, (m3 + m5) + _nn(ut[0:HT], tr))
            m4 = prod(4)
            m2 = prod(2)
            emit(HT, HT, n0, (m4 + m2) + _nn(ut[HT:T2], tl))
            m1 = prod(1)
            emit(0, HT, n0, ((m4 - m5) + m1) + prod(7) + _nn(ut[0:HT], tl))
            p22 = (m3 - m2) + m1
            ra = 0
            for rn in ([HT] if n0 == 0 else [256, 128, 128]):
                rs = slice(ra, ra + rn)
                emit(HT + ra, rn, HD + n0, p22[rs] + prod(6, rs) + _nn(ut[HT + ra:HT + ra + rn], tr))
                ra += rn

    def step(t, carry):
        pl.when(t == 0)(lambda: phase1(t))
        pl.when(t > 0)(lambda: phase2(t - 1))
        return carry

    lax.fori_loop(0, 1 + S // T2, step, 0)
    cp(o_ref, o_hbm, sem.at[2]).wait()


@jax.jit
def pallas_gated_mix__linear_kernel_hedgehog__mixer_s_mlp__prompt_kernel(
    A_x: jax.Array,
    A_wqkv: jax.Array,
    A_w_phi: jax.Array,
    A_wo: jax.Array,
    B_x: jax.Array,
    B_w1: jax.Array,
    B_w2: jax.Array,
    B_w3: jax.Array,
    B_w4: jax.Array,
    gate_w: jax.Array,
):
    del B_x
    x = A_x.reshape(S, D)
    wphi = jnp.transpose(A_w_phi, (1, 2, 0))
    w3t = B_w3.T
    hbm = pl.BlockSpec(memory_space=pl.ANY)
    out = pl.pallas_call(
        _kernel,
        in_specs=[hbm] * 9,
        out_specs=hbm,
        out_shape=jax.ShapeDtypeStruct((S, D), bf16),
        scratch_shapes=[
            pltpu.VMEM((S, D), bf16),
            pltpu.VMEM((D, 3 * D), bf16),
            pltpu.VMEM((DH, DH, H), bf16),
            pltpu.VMEM((D, D), bf16),
            pltpu.VMEM((D, D), bf16),
            pltpu.VMEM((D, D), bf16),
            pltpu.VMEM((F, D), bf16),
            pltpu.VMEM((F, D), bf16),
            pltpu.VMEM((D,), bf16),
            pltpu.VMEM((S, D), bf16),
            pltpu.VMEM((D // 2, D), u32),
            pltpu.VMEM((G, 64, 128), f32),
            pltpu.VMEM((G, 32, 128), u32),
            pltpu.VMEM((G, 128, 128), f32),
            pltpu.VMEM((4, S + 2 * PAD, 128), f32),
            pltpu.SemaphoreType.DMA((6,)),
        ],
        compiler_params=pltpu.CompilerParams(
            vmem_limit_bytes=100 * 1024 * 1024,
            disable_bounds_checks=True,
            disable_semaphore_checks=True,
        ),
    )(x, A_wqkv, wphi, A_wo, B_w1, B_w2, w3t, B_w4, gate_w)
    return out.reshape(1, S, D)
```

```python
import functools

import jax
import jax.numpy as jnp
from jax import lax
import jax.experimental.pallas as pl
import jax.experimental.pallas.tpu as pltpu

S, D, H, DH, F = 2048, 512, 32, 16, 1376
G = 8
FM = 1280
PAD = 8
T2 = 1024
XC = 768
HD, HF, HT = D // 2, FM // 2, T2 // 2
LOG2E = 1.4426950408889634

V0_ORDER = '5642713'
P1_SEQ = 'h6 v1 v2 v5 v3 h7 h4 h3 h2 v4 h5 v7 h1 v6'.split()
P2_SEQ = 'm5 q m3 m4 m7 m1 n m6 m2 o3 o1 o2 o4 o5 o7 o6 u4 u1 t u0 u2 u3'.split()
U_ORDERS = ('1235746', '1345726', '1435726', '1347256', '3564127')

f32 = jnp.float32
bf16 = jnp.bfloat16
u32 = jnp.uint32

_nn = functools.partial(jnp.dot, preferred_element_type=f32)
_nt = functools.partial(lax.dot_general, dimension_numbers=(((1,), (1,)), ((), ())),
                        preferred_element_type=f32)
_tn = functools.partial(lax.dot_general, dimension_numbers=(((0,), (0,)), ((), ())),
                        preferred_element_type=f32)


def _gelu(x):
    c = 0.7978845608028654
    inner = x * (c + (c * 0.044715) * (x * x))
    hx = 0.5 * x
    return hx + hx * jnp.tanh(inner)


def _ln_stats(x):
    m = jnp.mean(x, axis=-1, keepdims=True)
    xc = x - m
    v = jnp.mean(xc * xc, axis=-1, keepdims=True)
    return m, xc, lax.rsqrt(v + 1e-5)


def _fold4(v, op):
    return op(v, pltpu.roll(v, 4, 0))


def _exps(p):
    p3 = p.reshape(8, 8, p.shape[-1])
    mx = _fold4(jnp.max(p3, axis=0), jnp.maximum)
    mn = _fold4(jnp.min(p3, axis=0), jnp.minimum)
    ep = jnp.exp2(p3 - mx[None])
    en = jnp.exp2(mn[None] - p3)
    sp = _fold4(jnp.sum(ep, axis=0), jnp.add)
    sn = _fold4(jnp.sum(en, axis=0), jnp.add)
    return ep, en, sp, sn


def _left_ops(a11, a12, a21, a22):
    return [v.astype(bf16) for v in
            (a11 + a22, a21 + a22, a11, a22, a11 + a12, a21 - a11, a12 - a22)]


def _right_ops(read):
    f = lambda i, k: read(i, k).astype(f32)
    return [(f(0, 0) + f(3, 0)).astype(bf16), read(0, 1), (f(1, 2) - f(3, 2)).astype(bf16),
            (f(2, 3) - f(0, 3)).astype(bf16), read(3, 4), (f(0, 5) + f(1, 5)).astype(bf16),
            (f(2, 6) + f(3, 6)).astype(bf16)]


def _combine(m, order):
    pos = {int(k): i for i, k in enumerate(order)}

    def comb(terms):
        terms = sorted(terms, key=lambda t: pos[abs(t)])
        if terms[0] < 0:
            acc, rest = m[terms[1]] - m[-terms[0]], terms[2:]
        else:
            acc, rest = m[terms[0]], terms[1:]
        for t in rest:
            acc = acc + m[t] if t > 0 else acc - m[-t]
        return acc

    return comb([1, 4, -5, 7]), comb([3, 5]), comb([2, 4]), comb([1, -2, 3, 6])


def _strassen(mm, a, b, order):
    m = {}
    for k in order:
        m[int(k)] = mm(a[int(k) - 1], b[int(k) - 1])
    return _combine(m, order)


def _quad(v):
    r, c = v.shape[0] // 2, v.shape[1] // 2
    return v[0:r, 0:c], v[0:r, c:], v[r:, 0:c], v[r:, c:]


def _join(c11, c12, c21, c22):
    return jnp.concatenate([jnp.concatenate([c11, c12], axis=1),
                            jnp.concatenate([c21, c22], axis=1)], axis=0)


def _group(p, g):
    base = (g // 2) * 120
    last = p[base + 56:base + 64]
    low = lax.broadcasted_iota(jnp.int32, last.shape, 0) < 4
    if g % 2 == 0:
        return jnp.concatenate([p[base:base + 56], jnp.where(low, last, 0.0)], axis=0)
    return jnp.concatenate([jnp.where(low, 0.0, last), p[base + 64:base + 120]], axis=0)


def _iota(shape, dim):
    return lax.broadcasted_iota(jnp.int32, shape, dim)


def _kernel(x_hbm, wqkv_hbm, wphi_hbm, wo_hbm, w1_hbm, w2_hbm, w3t_hbm, w4_hbm, gw_hbm, o_hbm,
            x_ref, wqkv_ref, wphi_ref, wo_ref, w1_ref, w2_ref, w3t_ref, w4_ref, gw_ref, o_ref,
            wq_ref, kv_ref, kvb_ref, z_ref, h_ref, sem):
    cp = pltpu.make_async_copy
    lo_, hi_ = slice(0, HD), slice(HD, D)

    def w_cols(a, b, s):
        return cp(wqkv_hbm.at[:, a:b], wqkv_ref.at[:, a:b], sem.at[s])

    def x_rows(a, b, s):
        return cp(x_hbm.at[a:b, :], x_ref.at[a:b, :], sem.at[s])

    def start(cs):
        for c in cs:
            c.start()

    def wait(cs):
        for c in cs:
            c.wait()

    g0 = [cp(wphi_hbm, wphi_ref, sem.at[0])]
    g1 = [w_cols(D, D + 256, 1)]
    g2 = [x_rows(0, 128, 2)]
    g3 = [w_cols(D + 256, D + 384, 3), x_rows(128, 256, 3)]
    g4 = [w_cols(D + 384, 2 * D, 4), x_rows(256, 512, 4)]
    g5 = [w_cols(2 * D, 3 * D, 5), x_rows(512, XC, 5), cp(gw_hbm, gw_ref, sem.at[5])]
    g6 = [cp(w1_hbm, w1_ref, sem.at[0]), x_rows(XC, S, 0), w_cols(0, D, 0)]
    g7 = [cp(w2_hbm, w2_ref, sem.at[1]), cp(wo_hbm, wo_ref, sem.at[1]),
          cp(w3t_hbm, w3t_ref, sem.at[1]), cp(w4_hbm, w4_ref, sem.at[1])]
    start(g0 + g1 + g2 + g3 + g4 + g5)

    def right_ops(t, ref, blocks):
        def read(i, k):
            r, n, cols = blocks[i]
            return ref[pl.ds(pl.multiple_of((t >> (2 + k)) * 16 + r, 16), n), cols]
        return _right_ops(read)

    def phase1(t):
        h_ref[:, PAD:2 * PAD, :] = jnp.zeros((4, PAD, 128), f32)
        h_ref[:, S:PAD + S, :] = jnp.zeros((4, PAD, 128), f32)

        rep = jnp.where(_iota((32, 512), 0) == _iota((32, 512), 1) // 16, 1.0, 0.0).astype(bf16)
        lane_d = _iota((16, 512), 1) % 16
        low = _iota((8, 512), 0) < 4
        r = _iota((128, 128), 0)
        m2 = (r // 64) * 4 + r % 4 == _iota((128, 128), 1) // 16
        wait(g0)
        start(g6)
        w2d = wphi_ref[...].reshape(256, 32)
        cc = _nn(w2d, rep)
        e16 = cc[0:16, :]
        for d in range(1, DH):
            e16 = jnp.where(lane_d == d, cc[d * 16:(d + 1) * 16, :], e16)
        e64 = jnp.concatenate(
            [jnp.where(low, jnp.broadcast_to(e16[2 * i:2 * i + 1, :], (8, 512)),
                       jnp.broadcast_to(e16[2 * i + 1:2 * i + 2, :], (8, 512))) for i in range(8)], axis=0)
        et = jnp.concatenate([e64, e64], axis=0)
        bdt = jnp.where(jnp.concatenate([m2] * 4, axis=1), et, 0.0).astype(bf16)

        def fold(c0, b):
            lo = c0 + b * 128
            w = _nt(bdt[:, b * 128:(b + 1) * 128], wqkv_ref[:, lo:lo + 128]) * LOG2E
            la, lb = w[0:8], w[64:72]
            ra = jnp.where(low, pltpu.roll(la, 4, 0), la)
            rb = jnp.where(low, lb, pltpu.roll(lb, 4, 0))
            return jnp.concatenate([(w[8:64].reshape(7, 8, D) - ra[None]).reshape(56, D),
                                    jnp.where(low, la - ra, lb - rb),
                                    (w[72:128].reshape(7, 8, D) - rb[None]).reshape(56, D)], axis=0)

        def k_phi(kt):
            n = kt.shape[-1]
            ep, en, sp, sn = _exps(kt)
            rp = pl.reciprocal(sp, approx=True)
            rn = pl.reciprocal(sn, approx=True)
            phi = jnp.concatenate([(ep * rp[None]).reshape(64, n),
                                   (en * rn[None]).reshape(64, n)], axis=0)
            z = phi[:, 0:128]
            for c in range(1, n // 128):
                z = z + phi[:, c * 128:(c + 1) * 128]
            return phi, z

        def x_ops(c0, c1):
            n = (c1 - c0) // 2
            return right_ops(t, x_ref, [(c0, n, lo_), (c0 + n, n, lo_), (c0, n, hi_), (c0 + n, n, hi_)])

        wk = {}
        phis = {}
        z_set = set()
        pending = []

        def feat(g, c, kt):
            phi, z = k_phi(kt)
            if g in z_set:
                z_ref[g] += z
            else:
                z_ref[g] = z
                z_set.add(g)
            for j in range(kt.shape[1] // 128):
                phis[(g, c + j * 128)] = phi[:, j * 128:(j + 1) * 128].astype(bf16)

        def kproj(g_lo, g_hi, c0, c1, defer=False):
            w = jnp.concatenate([wk[b] for b in range(g_lo // 2, g_hi // 2)], axis=0)
            kt = _nt(w.astype(bf16), x_ref[c0:c1, :])
            n = c1 - c0
            for g in range(g_lo, g_hi):
                kg = _group(kt, g - g_lo)
                if defer:
                    if n > 128:
                        feat(g, c0, kg[:, 0:n - 128])
                    pending.append((g, c1 - 128, kg[:, n - 128:n]))
                else:
                    feat(g, c0, kg)

        wait(g1)
        wk[0] = fold(D, 0)
        wk[1] = fold(D, 1)
        wait(g2)
        kproj(0, 4, 0, 128, defer=True)
        wait(g3)
        wk[2] = fold(D, 2)
        kproj(0, 4, 128, 256)
        kproj(4, 6, 0, 256, defer=True)
        wait(g4)
        wk[3] = fold(D, 3)
        kproj(0, 6, 256, 512)
        kproj(6, 8, 0, 256)
        kproj(6, 8, 256, 512, defer=True)
        wait(g5)
        for p in pending:
            feat(*p)
        start(g7)
        wvq = _quad(wqkv_ref[:, 2 * D:3 * D].T.astype(f32))
        wva = _left_ops(*wvq)
        kproj(0, G, 512, XC)
        vt = _join(*_strassen(_nt, wva, x_ops(0, XC), V0_ORDER))
        for g in range(G):
            acc = None
            for c in range(0, XC, 128):
                pr = _nt(vt[g * 64:(g + 1) * 64, c:c + 128].astype(bf16), phis[(g, c)])
                acc = pr if acc is None else acc + pr
            kv_ref[g] = acc
        wait(g6)

        wkq = _quad(jnp.concatenate([wk[b] for b in range(4)], axis=0))
        kva = _left_ops(*[jnp.concatenate([a, b], axis=0) for a, b in zip(wkq, wvq)])
        w1q = _quad(w1_ref[...])
        hb = _right_ops(lambda i, k: w1q[i])
        ys = []
        for r0 in (0, S // 2):
            _, xc, rs = _ln_stats(x_ref[r0:r0 + S // 2, :].astype(f32))
            ys.append(xc * rs)
        ha = _left_ops(ys[0][:, lo_], ys[0][:, hi_], ys[1][:, lo_], ys[1][:, hi_])
        xb = x_ops(XC, S)
        vm, hm = {}, {}
        for op in P1_SEQ:
            k = int(op[1])
            if op[0] == 'v':
                vm[k] = _nt(kva[k - 1], xb[k - 1])
            else:
                hm[k] = _nn(ha[k - 1], hb[k - 1])
        for i, c in enumerate(_combine(hm, [op[1] for op in P1_SEQ if op[0] == 'h'])):
            h = _gelu(c)
            r0 = PAD + (i // 2) * (S // 2)
            for j in range(2):
                ch = (i % 2) * 2 + j
                rs = r0 + (1, -1, 2, -2)[ch]
                h_ref[ch, rs:rs + S // 2, :] = h[:, j * 128:(j + 1) * 128]
        wq_ref[...] = pltpu.bitcast(jnp.concatenate([fold(0, b) for b in range(4)], axis=0).astype(bf16), u32)
        cs = _combine(vm, [op[1] for op in P1_SEQ if op[0] == 'v'])
        kt = _join(*[c[0:240] for c in cs])
        vt = _join(*[c[240:240 + HD] for c in cs])
        phs = []
        for g in range(G):
            phi, z = k_phi(_group(kt, g))
            z_ref[g] += z
            phs.append(phi.astype(bf16))
        for g in range(G):
            kv_ref[g] += _nt(vt[g * 64:(g + 1) * 64, :].astype(bf16), phs[g])
        head_match = (_iota((64, 128), 0) // 16) == (_iota((64, 128), 1) % 4)
        for g in range(G):
            kvb_ref[g] = pltpu.bitcast(jnp.where(head_match, kv_ref[g], 0.0).astype(bf16), u32)
        wait(g7)

    def phase2(t):
        r0 = pl.multiple_of(t * T2, T2)
        x = x_ref[pl.ds(r0, T2), :]
        xf = x.astype(f32)
        gw = gw_ref[...].astype(f32).reshape(1, D)
        xg = x_ref[pl.ds(pl.multiple_of(r0 + (t >> 2) * 16, 16), T2), :].astype(f32)
        gate = 0.5 + 0.5 * jnp.tanh(0.5 * jnp.sum(xg * gw, axis=-1, keepdims=True))

        square = [(0, HD, lo_), (0, HD, hi_), (HD, HD, lo_), (HD, HD, hi_)]
        base = pl.multiple_of(PAD + t * T2, 8)
        hs = jnp.concatenate([h_ref[j, pl.ds(base, T2), :] for j in range(4)], axis=1)
        ha = _left_ops(*_quad(hs))
        hb = right_ops(t, w2_ref, square)
        ob = right_ops(t, wo_ref, square)
        mm, om, us, st = {}, {}, {}, {}

        def norm2():
            if 'y' not in st:
                x1 = xf + _join(*_combine(mm, [op[1] for op in P2_SEQ if op[0] == 'm']))
                m, _, rs = _ln_stats(x1)
                yf = x1 * rs - m * rs
                st['x1'], st['y'], st['ya'] = x1, yf.astype(bf16), _left_ops(*_quad(yf))
            return st

        for op in P2_SEQ:
            if op == 'q':
                qt = _nt(pltpu.bitcast(wq_ref[...], bf16), x)
            elif op == 'n':
                ots = []
                for g in range(G):
                    ep, en, sp, sn = _exps(_group(qt, g))
                    zb = jnp.broadcast_to(jnp.sum(z_ref[g], axis=-1, keepdims=True), (128, 128))
                    z = jnp.concatenate([zb] * (T2 // 128), axis=1).reshape(16, 8, T2)
                    dp = jnp.sum(ep * z[0:8], axis=0)
                    dn = jnp.sum(en * z[8:16], axis=0)
                    rr = 1.0 / (_fold4(dp * sn + dn * sp, jnp.add) + 1e-6 * (sp * sn))
                    phi = jnp.concatenate([(ep * (sn * rr)[None]).reshape(64, T2),
                                           (en * (sp * rr)[None]).reshape(64, T2)], axis=0).astype(bf16)
                    ots.append(_nn(pltpu.bitcast(kvb_ref[g], bf16), phi))
                t11, t21, t12, t22 = _quad(jnp.concatenate(ots, axis=0))
                oa = _left_ops(t11, t12, t21, t22)
            elif op == 't':
                ut = _gelu(_nt(w3t_ref[FM:F, :], norm2()['y'])).astype(bf16).T
            elif op[0] == 'm':
                k = int(op[1])
                mm[k] = _nn(ha[k - 1], hb[k - 1])
            elif op[0] == 'o':
                k = int(op[1])
                om[k] = _tn(oa[k - 1], ob[k - 1])
            elif op[0] == 'u':
                j = int(op[1])
                n0 = j * 128
                ub = right_ops(t, w3t_ref, [(n0, 128, lo_), (HF + n0, 128, lo_),
                                            (n0, 128, hi_), (HF + n0, 128, hi_)])
                us[j] = [_gelu(v) for v in _strassen(_nt, norm2()['ya'], ub, U_ORDERS[j])]
        a = _join(*_combine(om, [op[1] for op in P2_SEQ if op[0] == 'o']))
        x1 = st['x1']
        ua = _left_ops(*[jnp.concatenate([us[j][i] for j in range(5)], axis=1) for i in range(4)])

        def emit(ra, rn, c0, h2):
            cols = slice(c0, c0 + 128)
            rows = pl.ds(pl.multiple_of(r0 + ra, 128), rn)
            b = x1[ra:ra + rn, cols] + h2
            o_ref[rows, cols] = (b + gate[ra:ra + rn] * (a[ra:ra + rn, cols] - b)).astype(bf16)
            cp(o_ref.at[rows, cols], o_hbm.at[rows, cols], sem.at[2]).start()

        for n0 in (0, 128):
            cl, cr = slice(n0, n0 + 128), slice(HD + n0, HD + n0 + 128)
            wb = right_ops(t, w4_ref, [(0, HF, cl), (0, HF, cr), (HF, HF, cl), (HF, HF, cr)])
            tl, tr = w4_ref[FM:F, cl], w4_ref[FM:F, cr]
            prod = lambda k, rs=slice(0, HT): _nn(ua[k - 1][rs], wb[k - 1])
            m3 = prod(3)
            m5 = prod(5)
            emit(0, HT, HD + n0, (m3 + m5) + _nn(ut[0:HT], tr))
            m4 = prod(4)
            m2 = prod(2)
            emit(HT, HT, n0, (m4 + m2) + _nn(ut[HT:T2], tl))
            m1 = prod(1)
            emit(0, HT, n0, ((m4 - m5) + m1) + prod(7) + _nn(ut[0:HT], tl))
            p22 = (m3 - m2) + m1
            ra = 0
            for rn in ([HT] if n0 == 0 else [256, 128, 128]):
                rs = slice(ra, ra + rn)
                emit(HT + ra, rn, HD + n0, p22[rs] + prod(6, rs) + _nn(ut[HT + ra:HT + ra + rn], tr))
                ra += rn

    def step(t, carry):
        pl.when(t == 0)(lambda: phase1(t))
        pl.when(t > 0)(lambda: phase2(t - 1))
        return carry

    lax.fori_loop(0, 1 + S // T2, step, 0)
    cp(o_ref, o_hbm, sem.at[2]).wait()


@jax.jit
def pallas_gated_mix__linear_kernel_hedgehog__mixer_s_mlp__prompt_kernel(
    A_x: jax.Array,
    A_wqkv: jax.Array,
    A_w_phi: jax.Array,
    A_wo: jax.Array,
    B_x: jax.Array,
    B_w1: jax.Array,
    B_w2: jax.Array,
    B_w3: jax.Array,
    B_w4: jax.Array,
    gate_w: jax.Array,
):
    del B_x
    x = A_x.reshape(S, D)
    wphi = jnp.transpose(A_w_phi, (1, 2, 0))
    w3t = B_w3.T
    hbm = pl.BlockSpec(memory_space=pl.ANY)
    out = pl.pallas_call(
        _kernel,
        in_specs=[hbm] * 9,
        out_specs=hbm,
        out_shape=jax.ShapeDtypeStruct((S, D), bf16),
        scratch_shapes=[
            pltpu.VMEM((S, D), bf16),
            pltpu.VMEM((D, 3 * D), bf16),
            pltpu.VMEM((DH, DH, H), bf16),
            pltpu.VMEM((D, D), bf16),
            pltpu.VMEM((D, D), bf16),
            pltpu.VMEM((D, D), bf16),
            pltpu.VMEM((F, D), bf16),
            pltpu.VMEM((F, D), bf16),
            pltpu.VMEM((D,), bf16),
            pltpu.VMEM((S, D), bf16),
            pltpu.VMEM((240, D), u32),
            pltpu.VMEM((G, 64, 128), f32),
            pltpu.VMEM((G, 32, 128), u32),
            pltpu.VMEM((G, 128, 128), f32),
            pltpu.VMEM((4, S + 2 * PAD, 128), f32),
            pltpu.SemaphoreType.DMA((6,)),
        ],
        compiler_params=pltpu.CompilerParams(
            vmem_limit_bytes=100 * 1024 * 1024,
            disable_bounds_checks=True,
            disable_semaphore_checks=True,
        ),
    )(x, A_wqkv, wphi, A_wo, B_w1, B_w2, w3t, B_w4, gate_w)
    return out.reshape(1, S, D)
```

```python
import functools

import jax
import jax.numpy as jnp
from jax import lax
import jax.experimental.pallas as pl
import jax.experimental.pallas.tpu as pltpu

S, D, H, DH, F = 2048, 512, 32, 16, 1376
G = 8
FM = 1280
PAD = 8
T2 = 1024
XC = 768
HD, HF, HT = D // 2, FM // 2, T2 // 2
LOG2E = 1.4426950408889634

V0_ORDER = '5642713'
P1_SEQ = 'h7 v1 v2 v5 v3 h4 h3 h2 v4 h5 v7 h1 v6 h6'.split()
P2_SEQ = 'm5 q m3 m1 m7 m4 n m6 m2 o3 o1 o2 o4 o5 o7 o6 u4 u1 t u0 u2 u3'.split()
U_ORDERS = ('1235746', '1345726', '1435726', '1347256', '3564127')

f32 = jnp.float32
bf16 = jnp.bfloat16
u32 = jnp.uint32

_nn = functools.partial(jnp.dot, preferred_element_type=f32)
_nt = functools.partial(lax.dot_general, dimension_numbers=(((1,), (1,)), ((), ())),
                        preferred_element_type=f32)
_tn = functools.partial(lax.dot_general, dimension_numbers=(((0,), (0,)), ((), ())),
                        preferred_element_type=f32)


def _gelu(x):
    c = 0.7978845608028654
    inner = x * (c + (c * 0.044715) * (x * x))
    hx = 0.5 * x
    return hx + hx * jnp.tanh(inner)


def _ln_stats(x):
    m = jnp.mean(x, axis=-1, keepdims=True)
    xc = x - m
    v = jnp.mean(xc * xc, axis=-1, keepdims=True)
    return m, xc, lax.rsqrt(v + 1e-5)


def _fold4(v, op):
    return op(v, pltpu.roll(v, 4, 0))


def _exps(p):
    p3 = p.reshape(8, 8, p.shape[-1])
    mx = _fold4(jnp.max(p3, axis=0), jnp.maximum)
    mn = _fold4(jnp.min(p3, axis=0), jnp.minimum)
    ep = jnp.exp2(p3 - mx[None])
    en = jnp.exp2(mn[None] - p3)
    sp = _fold4(jnp.sum(ep, axis=0), jnp.add)
    sn = _fold4(jnp.sum(en, axis=0), jnp.add)
    return ep, en, sp, sn


def _left_ops(a11, a12, a21, a22):
    return [v.astype(bf16) for v in
            (a11 + a22, a21 + a22, a11, a22, a11 + a12, a21 - a11, a12 - a22)]


def _right_ops(read):
    f = lambda i, k: read(i, k).astype(f32)
    return [(f(0, 0) + f(3, 0)).astype(bf16), read(0, 1), (f(1, 2) - f(3, 2)).astype(bf16),
            (f(2, 3) - f(0, 3)).astype(bf16), read(3, 4), (f(0, 5) + f(1, 5)).astype(bf16),
            (f(2, 6) + f(3, 6)).astype(bf16)]


def _combine(m, order):
    pos = {int(k): i for i, k in enumerate(order)}

    def comb(terms):
        terms = sorted(terms, key=lambda t: pos[abs(t)])
        if terms[0] < 0:
            acc, rest = m[terms[1]] - m[-terms[0]], terms[2:]
        else:
            acc, rest = m[terms[0]], terms[1:]
        for t in rest:
            acc = acc + m[t] if t > 0 else acc - m[-t]
        return acc

    return comb([1, 4, -5, 7]), comb([3, 5]), comb([2, 4]), comb([1, -2, 3, 6])


def _strassen(mm, a, b, order):
    m = {}
    for k in order:
        m[int(k)] = mm(a[int(k) - 1], b[int(k) - 1])
    return _combine(m, order)


def _quad(v):
    r, c = v.shape[0] // 2, v.shape[1] // 2
    return v[0:r, 0:c], v[0:r, c:], v[r:, 0:c], v[r:, c:]


def _join(c11, c12, c21, c22):
    return jnp.concatenate([jnp.concatenate([c11, c12], axis=1),
                            jnp.concatenate([c21, c22], axis=1)], axis=0)


def _group(p, g):
    base = (g // 2) * 120
    last = p[base + 56:base + 64]
    low = lax.broadcasted_iota(jnp.int32, last.shape, 0) < 4
    if g % 2 == 0:
        return jnp.concatenate([p[base:base + 56], jnp.where(low, last, 0.0)], axis=0)
    return jnp.concatenate([jnp.where(low, 0.0, last), p[base + 64:base + 120]], axis=0)


def _iota(shape, dim):
    return lax.broadcasted_iota(jnp.int32, shape, dim)


def _kernel(x_hbm, wqkv_hbm, wphi_hbm, wo_hbm, w1_hbm, w2_hbm, w3t_hbm, w4_hbm, gw_hbm, o_hbm,
            x_ref, wqkv_ref, wphi_ref, wo_ref, w1_ref, w2_ref, w3t_ref, w4_ref, gw_ref, o_ref,
            wq_ref, kv_ref, kvb_ref, z_ref, h_ref, sem):
    cp = pltpu.make_async_copy
    lo_, hi_ = slice(0, HD), slice(HD, D)

    def w_cols(a, b, s):
        return cp(wqkv_hbm.at[:, a:b], wqkv_ref.at[:, a:b], sem.at[s])

    def x_rows(a, b, s):
        return cp(x_hbm.at[a:b, :], x_ref.at[a:b, :], sem.at[s])

    def start(cs):
        for c in cs:
            c.start()

    def wait(cs):
        for c in cs:
            c.wait()

    g0 = [cp(wphi_hbm, wphi_ref, sem.at[0])]
    g1 = [w_cols(D, D + 256, 1)]
    g2 = [x_rows(0, 128, 2)]
    g3 = [w_cols(D + 256, D + 384, 3), x_rows(128, 256, 3)]
    g4 = [w_cols(D + 384, 2 * D, 4), x_rows(256, 512, 4)]
    g5 = [w_cols(2 * D, 3 * D, 5), x_rows(512, XC, 5), cp(gw_hbm, gw_ref, sem.at[5])]
    g6 = [cp(w1_hbm, w1_ref, sem.at[0]), x_rows(XC, S, 0), w_cols(0, D, 0)]
    g7 = [cp(w2_hbm, w2_ref, sem.at[1]), cp(wo_hbm, wo_ref, sem.at[1]),
          cp(w3t_hbm, w3t_ref, sem.at[1]), cp(w4_hbm, w4_ref, sem.at[1])]
    start(g0 + g1 + g2 + g3 + g4 + g5)

    def right_ops(t, ref, blocks):
        def read(i, k):
            r, n, cols = blocks[i]
            return ref[pl.ds(pl.multiple_of((t >> (2 + k)) * 16 + r, 16), n), cols]
        return _right_ops(read)

    def phase1(t):
        h_ref[:, PAD:2 * PAD, :] = jnp.zeros((4, PAD, 128), f32)
        h_ref[:, S:PAD + S, :] = jnp.zeros((4, PAD, 128), f32)

        rep = jnp.where(_iota((32, 512), 0) == _iota((32, 512), 1) // 16, 1.0, 0.0).astype(bf16)
        lane_d = _iota((16, 512), 1) % 16
        low = _iota((8, 512), 0) < 4
        r = _iota((128, 128), 0)
        m2 = (r // 64) * 4 + r % 4 == _iota((128, 128), 1) // 16
        wait(g0)
        start(g6)
        w2d = wphi_ref[...].reshape(256, 32)
        cc = _nn(w2d, rep)
        e16 = cc[0:16, :]
        for d in range(1, DH):
            e16 = jnp.where(lane_d == d, cc[d * 16:(d + 1) * 16, :], e16)
        e64 = jnp.concatenate(
            [jnp.where(low, jnp.broadcast_to(e16[2 * i:2 * i + 1, :], (8, 512)),
                       jnp.broadcast_to(e16[2 * i + 1:2 * i + 2, :], (8, 512))) for i in range(8)], axis=0)
        et = jnp.concatenate([e64, e64], axis=0)
        bdt = jnp.where(jnp.concatenate([m2] * 4, axis=1), et, 0.0).astype(bf16)

        def fold(c0, b):
            lo = c0 + b * 128
            w = _nt(bdt[:, b * 128:(b + 1) * 128], wqkv_ref[:, lo:lo + 128]) * LOG2E
            la, lb = w[0:8], w[64:72]
            ra = jnp.where(low, pltpu.roll(la, 4, 0), la)
            rb = jnp.where(low, lb, pltpu.roll(lb, 4, 0))
            return jnp.concatenate([(w[8:64].reshape(7, 8, D) - ra[None]).reshape(56, D),
                                    jnp.where(low, la - ra, lb - rb),
                                    (w[72:128].reshape(7, 8, D) - rb[None]).reshape(56, D)], axis=0)

        def k_phi(kt):
            n = kt.shape[-1]
            ep, en, sp, sn = _exps(kt)
            phi = jnp.concatenate([(ep * pl.reciprocal(sp, approx=True)[None]).reshape(64, n),
                                   (en * pl.reciprocal(sn, approx=True)[None]).reshape(64, n)], axis=0)
            z = phi[:, 0:128]
            for c in range(1, n // 128):
                z = z + phi[:, c * 128:(c + 1) * 128]
            return phi, z

        def x_ops(c0, c1):
            n = (c1 - c0) // 2
            return right_ops(t, x_ref, [(c0, n, lo_), (c0 + n, n, lo_), (c0, n, hi_), (c0 + n, n, hi_)])

        wk = {}
        phis = {}
        z_set = set()
        pending = []

        def feat(g, c, kt):
            phi, z = k_phi(kt)
            if g in z_set:
                z_ref[g] += z
            else:
                z_ref[g] = z
                z_set.add(g)
            for j in range(kt.shape[1] // 128):
                phis[(g, c + j * 128)] = phi[:, j * 128:(j + 1) * 128].astype(bf16)

        def kproj(g_lo, g_hi, c0, c1, defer=False):
            w = jnp.concatenate([wk[b] for b in range(g_lo // 2, g_hi // 2)], axis=0)
            kt = _nt(w.astype(bf16), x_ref[c0:c1, :])
            n = c1 - c0
            for g in range(g_lo, g_hi):
                kg = _group(kt, g - g_lo)
                if defer:
                    if n > 128:
                        feat(g, c0, kg[:, 0:n - 128])
                    pending.append((g, c1 - 128, kg[:, n - 128:n]))
                else:
                    feat(g, c0, kg)

        wait(g1)
        wk[0] = fold(D, 0)
        wk[1] = fold(D, 1)
        wait(g2)
        kproj(0, 4, 0, 128, defer=True)
        wait(g3)
        wk[2] = fold(D, 2)
        kproj(0, 4, 128, 256)
        kproj(4, 6, 0, 256, defer=True)
        wait(g4)
        wk[3] = fold(D, 3)
        kproj(0, 6, 256, 512)
        kproj(6, 8, 0, 256)
        kproj(6, 8, 256, 512, defer=True)
        wait(g5)
        for p in pending:
            feat(*p)
        start(g7)
        wvq = _quad(wqkv_ref[:, 2 * D:3 * D].T.astype(f32))
        wva = _left_ops(*wvq)
        kproj(0, G, 512, XC)
        vt = _join(*_strassen(_nt, wva, x_ops(0, XC), V0_ORDER))
        for g in range(G):
            acc = None
            for c in range(0, XC, 128):
                pr = _nt(vt[g * 64:(g + 1) * 64, c:c + 128].astype(bf16), phis[(g, c)])
                acc = pr if acc is None else acc + pr
            kv_ref[g] = acc
        wait(g6)

        wkq = _quad(jnp.concatenate([wk[b] for b in range(4)], axis=0))
        kva = _left_ops(*[jnp.concatenate([a, b], axis=0) for a, b in zip(wkq, wvq)])
        w1q = _quad(w1_ref[...])
        hb = _right_ops(lambda i, k: w1q[i])
        ys = []
        for r0 in (0, S // 2):
            _, xc, rs = _ln_stats(x_ref[r0:r0 + S // 2, :].astype(f32))
            ys.append(xc * rs)
        ha = _left_ops(ys[0][:, lo_], ys[0][:, hi_], ys[1][:, lo_], ys[1][:, hi_])
        xb = x_ops(XC, S)
        vm, hm = {}, {}
        for op in P1_SEQ:
            k = int(op[1])
            if op[0] == 'v':
                vm[k] = _nt(kva[k - 1], xb[k - 1])
            else:
                hm[k] = _nn(ha[k - 1], hb[k - 1])
        for i, c in enumerate(_combine(hm, [op[1] for op in P1_SEQ if op[0] == 'h'])):
            h = _gelu(c)
            r0 = PAD + (i // 2) * (S // 2)
            for j in range(2):
                ch = (i % 2) * 2 + j
                rs = r0 + (1, -1, 2, -2)[ch]
                h_ref[ch, rs:rs + S // 2, :] = h[:, j * 128:(j + 1) * 128]
        wq_ref[...] = pltpu.bitcast(jnp.concatenate([fold(0, b) for b in range(4)], axis=0).astype(bf16), u32)
        cs = _combine(vm, [op[1] for op in P1_SEQ if op[0] == 'v'])
        kt = _join(*[c[0:240] for c in cs])
        vt = _join(*[c[240:240 + HD] for c in cs])
        phs = []
        for g in range(G):
            phi, z = k_phi(_group(kt, g))
            z_ref[g] += z
            phs.append(phi.astype(bf16))
        for g in range(G):
            kv_ref[g] += _nt(vt[g * 64:(g + 1) * 64, :].astype(bf16), phs[g])
        head_match = (_iota((64, 128), 0) // 16) == (_iota((64, 128), 1) % 4)
        for g in range(G):
            kvb_ref[g] = pltpu.bitcast(jnp.where(head_match, kv_ref[g], 0.0).astype(bf16), u32)
        wait(g7)

    def phase2(t):
        r0 = pl.multiple_of(t * T2, T2)
        x = x_ref[pl.ds(r0, T2), :]
        xf = x.astype(f32)
        gw = gw_ref[...].astype(f32).reshape(1, D)
        xg = x_ref[pl.ds(pl.multiple_of(r0 + (t >> 2) * 16, 16), T2), :].astype(f32)
        gate = 0.5 + 0.5 * jnp.tanh(0.5 * jnp.sum(xg * gw, axis=-1, keepdims=True))

        square = [(0, HD, lo_), (0, HD, hi_), (HD, HD, lo_), (HD, HD, hi_)]
        base = pl.multiple_of(PAD + t * T2, 8)
        hs = jnp.concatenate([h_ref[j, pl.ds(base, T2), :] for j in range(4)], axis=1)
        ha = _left_ops(*_quad(hs))
        hb = right_ops(t, w2_ref, square)
        ob = right_ops(t, wo_ref, square)
        mm, om, us, st = {}, {}, {}, {}

        def norm2():
            if 'y' not in st:
                x1 = xf + _join(*_combine(mm, [op[1] for op in P2_SEQ if op[0] == 'm']))
                m, _, rs = _ln_stats(x1)
                yf = x1 * rs - m * rs
                st['x1'], st['y'], st['ya'] = x1, yf.astype(bf16), _left_ops(*_quad(yf))
            return st

        for op in P2_SEQ:
            if op == 'q':
                qt = _nt(pltpu.bitcast(wq_ref[...], bf16), x)
            elif op == 'n':
                ots = []
                for g in range(G):
                    ep, en, sp, sn = _exps(_group(qt, g))
                    zb = jnp.broadcast_to(jnp.sum(z_ref[g], axis=-1, keepdims=True), (128, 128))
                    z = jnp.concatenate([zb] * (T2 // 128), axis=1).reshape(16, 8, T2)
                    dp = jnp.sum(ep * z[0:8], axis=0)
                    dn = jnp.sum(en * z[8:16], axis=0)
                    rr = 1.0 / (_fold4(dp * sn + dn * sp, jnp.add) + 1e-6 * (sp * sn))
                    phi = jnp.concatenate([(ep * (sn * rr)[None]).reshape(64, T2),
                                           (en * (sp * rr)[None]).reshape(64, T2)], axis=0).astype(bf16)
                    ots.append(_nn(pltpu.bitcast(kvb_ref[g], bf16), phi))
                t11, t21, t12, t22 = _quad(jnp.concatenate(ots, axis=0))
                oa = _left_ops(t11, t12, t21, t22)
            elif op == 't':
                ut = _gelu(_nt(w3t_ref[FM:F, :], norm2()['y'])).astype(bf16).T
            elif op[0] == 'm':
                k = int(op[1])
                mm[k] = _nn(ha[k - 1], hb[k - 1])
            elif op[0] == 'o':
                k = int(op[1])
                om[k] = _tn(oa[k - 1], ob[k - 1])
            elif op[0] == 'u':
                j = int(op[1])
                n0 = j * 128
                ub = right_ops(t, w3t_ref, [(n0, 128, lo_), (HF + n0, 128, lo_),
                                            (n0, 128, hi_), (HF + n0, 128, hi_)])
                us[j] = [_gelu(v) for v in _strassen(_nt, norm2()['ya'], ub, U_ORDERS[j])]
        a = _join(*_combine(om, [op[1] for op in P2_SEQ if op[0] == 'o']))
        x1 = st['x1']
        ua = _left_ops(*[jnp.concatenate([us[j][i] for j in range(5)], axis=1) for i in range(4)])

        def emit(ra, rn, c0, h2):
            cols = slice(c0, c0 + 128)
            rows = pl.ds(pl.multiple_of(r0 + ra, 128), rn)
            b = x1[ra:ra + rn, cols] + h2
            o_ref[rows, cols] = (b + gate[ra:ra + rn] * (a[ra:ra + rn, cols] - b)).astype(bf16)
            cp(o_ref.at[rows, cols], o_hbm.at[rows, cols], sem.at[2]).start()

        for n0 in (0, 128):
            cl, cr = slice(n0, n0 + 128), slice(HD + n0, HD + n0 + 128)
            wb = right_ops(t, w4_ref, [(0, HF, cl), (0, HF, cr), (HF, HF, cl), (HF, HF, cr)])
            tl, tr = w4_ref[FM:F, cl], w4_ref[FM:F, cr]
            prod = lambda k, rs=slice(0, HT): _nn(ua[k - 1][rs], wb[k - 1])
            m3 = prod(3)
            m5 = prod(5)
            emit(0, HT, HD + n0, (m3 + m5) + _nn(ut[0:HT], tr))
            m4 = prod(4)
            m2 = prod(2)
            emit(HT, HT, n0, (m4 + m2) + _nn(ut[HT:T2], tl))
            m1 = prod(1)
            emit(0, HT, n0, ((m4 - m5) + m1) + prod(7) + _nn(ut[0:HT], tl))
            p22 = (m3 - m2) + m1
            ra = 0
            for rn in ([HT] if n0 == 0 else [256, 128, 128]):
                rs = slice(ra, ra + rn)
                emit(HT + ra, rn, HD + n0, p22[rs] + prod(6, rs) + _nn(ut[HT + ra:HT + ra + rn], tr))
                ra += rn

    def step(t, carry):
        pl.when(t == 0)(lambda: phase1(t))
        pl.when(t > 0)(lambda: phase2(t - 1))
        return carry

    lax.fori_loop(0, 1 + S // T2, step, 0)
    cp(o_ref, o_hbm, sem.at[2]).wait()


@jax.jit
def pallas_gated_mix__linear_kernel_hedgehog__mixer_s_mlp__prompt_kernel(
    A_x: jax.Array,
    A_wqkv: jax.Array,
    A_w_phi: jax.Array,
    A_wo: jax.Array,
    B_x: jax.Array,
    B_w1: jax.Array,
    B_w2: jax.Array,
    B_w3: jax.Array,
    B_w4: jax.Array,
    gate_w: jax.Array,
):
    del B_x
    x = A_x.reshape(S, D)
    wphi = jnp.transpose(A_w_phi, (1, 2, 0))
    w3t = B_w3.T
    hbm = pl.BlockSpec(memory_space=pl.ANY)
    out = pl.pallas_call(
        _kernel,
        in_specs=[hbm] * 9,
        out_specs=hbm,
        out_shape=jax.ShapeDtypeStruct((S, D), bf16),
        scratch_shapes=[
            pltpu.VMEM((S, D), bf16),
            pltpu.VMEM((D, 3 * D), bf16),
            pltpu.VMEM((DH, DH, H), bf16),
            pltpu.VMEM((D, D), bf16),
            pltpu.VMEM((D, D), bf16),
            pltpu.VMEM((D, D), bf16),
            pltpu.VMEM((F, D), bf16),
            pltpu.VMEM((F, D), bf16),
            pltpu.VMEM((D,), bf16),
            pltpu.VMEM((S, D), bf16),
            pltpu.VMEM((240, D), u32),
            pltpu.VMEM((G, 64, 128), f32),
            pltpu.VMEM((G, 32, 128), u32),
            pltpu.VMEM((G, 128, 128), f32),
            pltpu.VMEM((4, S + 2 * PAD, 128), f32),
            pltpu.SemaphoreType.DMA((6,)),
        ],
        compiler_params=pltpu.CompilerParams(
            vmem_limit_bytes=100 * 1024 * 1024,
            disable_bounds_checks=True,
            disable_semaphore_checks=True,
        ),
    )(x, A_wqkv, wphi, A_wo, B_w1, B_w2, w3t, B_w4, gate_w)
    return out.reshape(1, S, D)
```
